```python
import jax
import jax.numpy as jnp

def _softmax(x, axis=-1):
    return jax.nn.softmax(x, axis=axis)

def _gelu(x):
    return jax.nn.gelu(x, approximate=True)

def _silu(x):
    return jax.nn.silu(x)

def _sigmoid(x):
    return jax.nn.sigmoid(x)

def _layernorm(x, axis=-1, eps=1e-05):
    m = jnp.mean(x, axis=axis, keepdims=True)
    v = jnp.var(x, axis=axis, keepdims=True)
    return (x - m) / jnp.sqrt(v + eps)

def _scatter_add(tgt, idx, src, axis=0):
    return tgt.at[idx].add(src)

def _segment_sum(src, seg, n):
    return jax.ops.segment_sum(src, seg, n)

class _Rng:

    def __init__(self, key):
        self._k = key

    def _next(self):
        self._k, sub = jax.random.split(self._k)
        return sub

    def normal(self, shape):
        return jax.random.normal(self._next(), shape, dtype=jnp.bfloat16)

    def randint(self, lo, hi, shape):
        return jax.random.randint(self._next(), shape, lo, hi, dtype=jnp.int32)

    def uniform(self, shape, lo=0.0, hi=1.0):
        return jax.random.uniform(self._next(), shape, jnp.bfloat16, lo, hi)

    def permutation(self, n):
        return jax.random.permutation(self._next(), n)
kernel_name = 'adaLN_cond__sliding_block_cached__dense_activation_gelu__decode'

def setup_inputs():
    _rng = _Rng(jax.random.key(int.from_bytes(__import__("os").urandom(4), "little")))
    _w = lambda a: (lambda t: t.astype(jnp.bfloat16) if jnp.issubdtype(t.dtype, jnp.floating) else t)(jnp.asarray(a))

    def _A_setup():
        B, Sq, D = (4, 1, 640)
        Hq, Hkv, Sk, Dh = (32, 32, 8192, 128)
        assert Hq % Hkv == 0, (Hq, Hkv)
        return {'x': _w((lambda *s: _rng.normal(s) * 0.05)(B, Sq, D)), 'k_cache': _w((lambda *s: _rng.normal(s) * 0.05)(B, Hkv, Sk, Dh)), 'v_cache': _w((lambda *s: _rng.normal(s) * 0.05)(B, Hkv, Sk, Dh)), 'wq': _w((lambda *s: _rng.normal(s) * 0.05)(D, Hq * Dh) * D ** (-0.5)), 'wo': _w((lambda *s: _rng.normal(s) * 0.05)(Hq * Dh, D) * (Hq * Dh) ** (-0.5))}
    _A_in = _A_setup()

    def _B_setup():
        B, S, D, F = (4, 1, 640, 1728)
        return {'x': _w((lambda *s: _rng.normal(s) * 0.05)(B, S, D)), 'w1': _w((lambda *s: _rng.normal(s) * 0.05)(D, F) * D ** (-0.5)), 'b1': _w((lambda *s: _rng.normal(s) * 0.05)(F) * 0.01), 'w2': _w((lambda *s: _rng.normal(s) * 0.05)(F, D) * F ** (-0.5)), 'b2': _w((lambda *s: _rng.normal(s) * 0.05)(D) * 0.01)}
    _B_in = _B_setup()
    return {'A_x': _A_in['x'], 'A_k_cache': _A_in['k_cache'], 'A_v_cache': _A_in['v_cache'], 'A_wq': _A_in['wq'], 'A_wo': _A_in['wo'], 'B_x': _B_in['x'], 'B_w1': _B_in['w1'], 'B_b1': _B_in['b1'], 'B_w2': _B_in['w2'], 'B_b2': _B_in['b2'], 'c': _w((lambda *s: _rng.normal(s) * 0.05)(4, 640)), 'w_mod': _w((lambda *s: _rng.normal(s) * 0.05)(640, 6 * 640) * 640 ** (-0.5))}

def reference(A_x, A_k_cache, A_v_cache, A_wq, A_wo, B_x, B_w1, B_b1, B_w2, B_b2, c, w_mod):

    def _A_ref(x, k_cache, v_cache, wq, wo):
        B, Sq, D = x.shape
        Hq, Dh = (32, 128)
        Hkv, Sk = (k_cache.shape[1], k_cache.shape[2])
        W = min(4096, max(256, Sk // 4))
        rep = Hq // Hkv
        q = (lambda x, *d: x.transpose(*d))((x @ wq).reshape(B, Sq, Hq, Dh), 0, 2, 1, 3)
        k = jnp.repeat(k_cache[:, :, Sk - W:, :], rep, axis=1)
        v = jnp.repeat(v_cache[:, :, Sk - W:, :], rep, axis=1)
        scores = jnp.einsum('bhqd,bhkd->bhqk', q, k) * Dh ** (-0.5)
        p = _softmax(scores, axis=-1)
        o = jnp.einsum('bhqk,bhkd->bhqd', p, v)
        return (lambda x, *d: x.transpose(*d))(o, 0, 2, 1, 3).reshape(B, Sq, Hq * Dh) @ wo

    def _B_ref(x, w1, b1, w2, b2):
        h = jnp.einsum('bsd,df->bsf', x, w1) + b1
        h = _gelu(h)
        return jnp.einsum('bsf,fd->bsd', h, w2) + b2
    x = A_x
    mod = (_silu(c) @ w_mod).reshape(c.shape[0], 6, 1, -1)
    sa, ca, ga, sb, cb, gb = (mod[:, 0].copy(), mod[:, 1].copy(), mod[:, 2].copy(), mod[:, 3].copy(), mod[:, 4].copy(), mod[:, 5].copy())
    h = _layernorm(x, axis=-1) * (1 + ca) + sa
    x = x + ga * _A_ref(h, A_k_cache, A_v_cache, A_wq, A_wo)
    h = _layernorm(x, axis=-1) * (1 + cb) + sb
    x = x + gb * _B_ref(h, B_w1, B_b1, B_w2, B_b2)
    return x
```

```python
import jax
import jax.numpy as jnp
from jax import lax
import jax.experimental.pallas as pl
import jax.experimental.pallas.tpu as pltpu

F32 = jnp.float32
BF16 = jnp.bfloat16

_NT = (((1,), (1,)), ((), ()))


def _layernorm(x, eps=1e-5):
    m = jnp.mean(x, axis=-1, keepdims=True)
    d = x - m
    v = jnp.mean(d * d, axis=-1, keepdims=True)
    return d * lax.rsqrt(v + eps)


def _build(B, D, H, Sk, Dh, F, *, R, LA, NK, NV):
    W = min(4096, max(256, Sk // 4))
    OFF = Sk - W
    GH = 8
    NHG = H // GH
    NG = NHG * B
    CPG = W // R
    NU = NG * CPG
    DR = 16
    DPC = R // DR
    WR = 32
    scale = float(Dh) ** -0.5
    n_wo = H * Dh // WR
    n_f = F // WR
    wo_per_unit = n_wo // LA
    assert n_wo % (2 * LA) == 0 and n_f % 2 == 0

    def kernel(x_hbm, k_hbm, v_hbm, wq_hbm, wo_hbm, w1_hbm, b1_hbm, w2_hbm, b2_hbm, c_hbm, wm_hbm,
               out_ref,
               x_v, c_v, b1_v, b2_v, wm_v, wq_v, wo_v, w1_v, w2_v, kbuf, vbuf,
               q_scr, s_scr, p_scr, o_scr,
               sem_s, sem_w, sem_k, sem_v):
        small = [pltpu.make_async_copy(x_hbm, x_v, sem_s.at[0]),
                 pltpu.make_async_copy(c_hbm, c_v, sem_s.at[1]),
                 pltpu.make_async_copy(b1_hbm, b1_v, sem_s.at[2]),
                 pltpu.make_async_copy(b2_hbm, b2_v, sem_s.at[3])]

        def wait_region(ref, sem):
            pltpu.make_async_copy(ref, ref, sem).wait()

        def kv_copy(hbm, buf, sem, u, slot, d):
            g = u // CPG
            cj = u % CPG
            hg = g // B
            b = g % B
            r0 = pl.multiple_of(OFF + cj * R + d * DR, DR)
            return pltpu.make_async_copy(
                hbm.at[b, pl.ds(hg * GH, GH), pl.ds(r0, DR), :],
                buf.at[slot, :, pl.ds(d * DR, DR), :],
                sem.at[slot])

        def issue_kv(u):
            ks = u % NK
            vs = u % NV
            for d in range(DPC):
                kv_copy(k_hbm, kbuf, sem_k, u, ks, d).start(priority=0)
                kv_copy(v_hbm, vbuf, sem_v, u, vs, d).start(priority=1)

        def box_copy(hbm, buf, i, j, sem):
            sl = (pl.ds(i * 128, 128), pl.ds(j * 128, 128))
            return pltpu.make_async_copy(hbm.at[sl], buf.at[sl], sem)

        def row_copy(hbm, buf, i, sem):
            r0 = i * WR
            if not isinstance(r0, int):
                r0 = pl.multiple_of(r0, WR)
            return pltpu.make_async_copy(hbm.at[pl.ds(r0, WR), :], buf.at[pl.ds(r0, WR), :], sem)

        SEM_WMA, SEM_WMB, SEM_WQ, SEM_WO, SEM_W1, SEM_W2A, SEM_W2B = range(7)

        for cp in small:
            cp.start()
        nd = D // 128
        wm_list = [(i, j) for j in range(6 * nd) for i in range(nd)]
        wq_list = [(i, j) for j in range(H * Dh // 128) for i in range(nd)]
        for t in range(max(len(wm_list), len(wq_list))):
            if t < len(wm_list):
                i, j = wm_list[t]
                box_copy(wm_hbm, wm_v, i, j,
                         sem_w.at[SEM_WMA if j < 2 * nd else SEM_WMB]).start(priority=0)
                i, j = wq_list[t]
                box_copy(wq_hbm, wq_v, i, j, sem_w.at[SEM_WQ]).start(priority=1)
            else:
                i, j = wq_list[t]
                box_copy(wq_hbm, wq_v, i, j, sem_w.at[SEM_WQ]).start(priority=t % 2)

        small[0].wait()
        small[1].wait()
        x = x_v[...].astype(F32)
        sc = jax.nn.silu(c_v[...].astype(F32)).astype(BF16)
        wait_region(wm_v.at[:, pl.ds(0, 2 * D)], sem_w.at[SEM_WMA])
        mod_a = jnp.dot(sc, wm_v[:, 0:2 * D], preferred_element_type=F32)
        h = (_layernorm(x) * (1.0 + mod_a[:, D:2 * D]) + mod_a[:, 0:D]).astype(BF16)
        issue_kv(0)
        wait_region(wm_v.at[:, pl.ds(2 * D, 4 * D)], sem_w.at[SEM_WMB])
        mod_b = jnp.dot(sc, wm_v[:, 2 * D:6 * D], preferred_element_type=F32)
        issue_kv(1)
        wait_region(wq_v, sem_w.at[SEM_WQ])
        for hg in range(NHG):
            qq = jnp.dot(h, wq_v[:, hg * GH * Dh:(hg + 1) * GH * Dh], preferred_element_type=F32)
            qq = qq.astype(BF16).astype(F32)
            for j in range(GH):
                q_scr[pl.ds(hg * B * GH + j, B, stride=GH), :] = qq[:, j * Dh:(j + 1) * Dh]
            if 2 + hg < LA:
                issue_kv(2 + hg)
        for u in range(2 + NHG, LA):
            issue_kv(u)

        row = lax.broadcasted_iota(jnp.int32, (GH, Dh), 0)

        def qk(u, g, cj):
            slot = u % NK
            wait_region(kbuf.at[slot], sem_k.at[slot])
            qg = q_scr[pl.ds(pl.multiple_of(g * GH, GH), GH), :]
            s = None
            for j in range(GH):
                qm = jnp.where(row == j, qg, 0.0).astype(BF16)
                t = lax.dot_general(qm, kbuf[slot, j], _NT, preferred_element_type=F32)
                s = t if s is None else s + t
            s_scr[cj] = s

        def pv(u, cj, acc):
            slot = u % NV
            wait_region(vbuf.at[slot], sem_v.at[slot])
            p = p_scr[cj].astype(BF16)
            for j in range(GH):
                t = jnp.dot(p, vbuf[slot, j], preferred_element_type=F32)
                acc = acc + jnp.where(row == j, t, 0.0)
            return acc

        def softmax():
            s = s_scr[...] * scale
            m = jnp.max(jnp.max(s, axis=0), axis=-1, keepdims=True)
            p = jnp.exp(s - m[None])
            p_scr[...] = p
            return jnp.sum(jnp.sum(p, axis=0), axis=-1, keepdims=True)

        def issue_next(u):
            n = u + LA

            @pl.when(n < NU)
            def _():
                issue_kv(n)

            @pl.when(n >= NU)
            def _():
                base = (n - NU) * (wo_per_unit // 2)
                for d in range(wo_per_unit // 2):
                    row_copy(wo_hbm, wo_v, base + d, sem_w.at[SEM_WO]).start(priority=0)
                    row_copy(wo_hbm, wo_v, n_wo // 2 + base + d, sem_w.at[SEM_WO]).start(priority=1)

        def first_unit(cj, _):
            issue_next(cj)
            qk(cj, 0, cj)
            return 0

        lax.fori_loop(0, CPG, first_unit, 0)
        l0 = softmax()

        def group(g, l_prev):
            def unit(cj, acc):
                u = g * CPG + cj
                issue_next(u)
                qk(u, g, cj)
                return pv(u - CPG, cj, acc)

            acc = lax.fori_loop(0, CPG, unit, jnp.zeros((GH, Dh), F32))
            o_scr[pl.ds(pl.multiple_of((g - 1) * GH, GH), GH), :] = acc / l_prev
            return softmax()

        l_last = lax.fori_loop(1, NG, group, l0)

        def issue_f(hbm, buf, lo, hi, sem_lo, sem_hi):
            for i in range(lo, hi):
                row_copy(hbm, buf, i, sem_lo).start(priority=0)
                row_copy(hbm, buf, n_f // 2 + i, sem_hi).start(priority=1)

        hf = n_f // 2
        acc = jnp.zeros((GH, Dh), F32)
        for cj in range(CPG):
            acc = pv(NU - CPG + cj, cj, acc)
            if cj == CPG // 2 - 1:
                issue_f(w1_hbm, w1_v, 0, hf // 2, sem_w.at[SEM_W1], sem_w.at[SEM_W1])
        o_scr[pl.ds((NG - 1) * GH, GH), :] = acc / l_last
        issue_f(w1_hbm, w1_v, hf // 2, hf, sem_w.at[SEM_W1], sem_w.at[SEM_W1])

        wait_region(wo_v, sem_w.at[SEM_WO])
        issue_f(w2_hbm, w2_v, 0, hf // 2, sem_w.at[SEM_W2A], sem_w.at[SEM_W2A])
        attn = None
        for hg in range(NHG):
            o = jnp.concatenate(
                [o_scr[pl.ds(hg * B * GH + j, B, stride=GH), :] for j in range(GH)], axis=1)
            t = jnp.dot(o.astype(BF16), wo_v[hg * GH * Dh:(hg + 1) * GH * Dh, :],
                        preferred_element_type=F32)
            attn = t if attn is None else attn + t
        issue_f(w2_hbm, w2_v, hf // 2, hf, sem_w.at[SEM_W2B], sem_w.at[SEM_W2B])

        ga, sb, cb, gb = (mod_b[:, i * D:(i + 1) * D] for i in range(4))
        x1 = x + ga * attn
        h2 = (_layernorm(x1) * (1.0 + cb) + sb).astype(BF16)
        small[2].wait()
        small[3].wait()
        b1 = b1_v[...].astype(F32).reshape(1, F)
        b2 = b2_v[...].astype(F32).reshape(1, D)
        wait_region(w1_v, sem_w.at[SEM_W1])
        f1 = lax.dot_general(h2, w1_v[...], _NT, preferred_element_type=F32) + b1
        f1 = jax.nn.gelu(f1, approximate=True).astype(BF16)

        a = (hf // 2) * WR
        half = hf * WR
        wait_region(w2_v.at[pl.ds(0, 2 * a), :], sem_w.at[SEM_W2A])
        wait_region(w2_v.at[pl.ds(0, F - 2 * a), :], sem_w.at[SEM_W2B])
        y = jnp.dot(f1, w2_v[...], preferred_element_type=F32) + b2
        out_ref[...] = (x1 + gb * y).astype(out_ref.dtype)

    scratch = [
        pltpu.VMEM((B, D), BF16), pltpu.VMEM((B, D), BF16),
        pltpu.VMEM((F,), BF16), pltpu.VMEM((D,), BF16),
        pltpu.VMEM((D, 6 * D), BF16), pltpu.VMEM((D, H * Dh), BF16),
        pltpu.VMEM((H * Dh, D), BF16), pltpu.VMEM((F, D), BF16), pltpu.VMEM((F, D), BF16),
        pltpu.VMEM((NK, GH, R, Dh), BF16), pltpu.VMEM((NV, GH, R, Dh), BF16),
        pltpu.VMEM((NG * GH, Dh), F32), pltpu.VMEM((CPG, GH, R), F32),
        pltpu.VMEM((CPG, GH, R), F32), pltpu.VMEM((NG * GH, Dh), F32),
        pltpu.SemaphoreType.DMA((4,)), pltpu.SemaphoreType.DMA((7,)),
        pltpu.SemaphoreType.DMA((NK,)), pltpu.SemaphoreType.DMA((NV,)),
    ]
    return kernel, scratch


@jax.jit
def pallas_adaLN_cond__sliding_block_cached__dense_activation_gelu__decode_kernel(
    A_x: jax.Array,
    A_k_cache: jax.Array,
    A_v_cache: jax.Array,
    A_wq: jax.Array,
    A_wo: jax.Array,
    B_x: jax.Array,
    B_w1: jax.Array,
    B_b1: jax.Array,
    B_w2: jax.Array,
    B_b2: jax.Array,
    c: jax.Array,
    w_mod: jax.Array,
):
    B, _, D = A_x.shape
    _, H, Sk, Dh = A_k_cache.shape
    F = B_w1.shape[1]
    kernel, scratch = _build(B, D, H, Sk, Dh, F, R=256, LA=4, NK=8, NV=16)
    out = pl.pallas_call(
        kernel,
        in_specs=[pl.BlockSpec(memory_space=pl.ANY)] * 11,
        out_specs=pl.BlockSpec(memory_space=pltpu.VMEM),
        out_shape=jax.ShapeDtypeStruct((B, D), A_x.dtype),
        scratch_shapes=scratch,
        compiler_params=pltpu.CompilerParams(
            vmem_limit_bytes=100 * 1024 * 1024, disable_bounds_checks=True),
    )(A_x.reshape(B, D), A_k_cache, A_v_cache, A_wq, A_wo, B_w1.T, B_b1, B_w2, B_b2, c, w_mod)
    return out.reshape(B, 1, D)
```

```python
import functools

import jax
import jax.numpy as jnp
from jax import lax
import jax.experimental.pallas as pl
import jax.experimental.pallas.tpu as pltpu

F32 = jnp.float32
BF16 = jnp.bfloat16

_NT = (((1,), (1,)), ((), ()))


def _layernorm(x, eps=1e-5):
    m = jnp.mean(x, axis=-1, keepdims=True)
    d = x - m
    v = jnp.mean(d * d, axis=-1, keepdims=True)
    return d * lax.rsqrt(v + eps)


def _build(B, D, H, Sk, Dh, F, *, R, LA, NK, NV, compute=True, HN=4, WON=8, WOR=32, FR=32, FA=896,
           W2B=(1280, 1536, 1728), scopes=False, diag=0, SH=24, KP=1):
    W = min(4096, max(256, Sk // 4))
    OFF = Sk - W
    GH = 8
    NHG = H // GH
    NG = NHG * B
    CPG = W // R
    NU = NG * CPG
    DR = 16
    DPC = R // DR
    scale = float(Dh) ** -0.5
    assert LA >= 3 and NK > LA and NV >= CPG + LA + 1 and 0 <= SH <= 2 * DPC
    n_wo = H * Dh // (2 * WOR)
    ND = NU * DPC
    assert SH <= n_wo
    assert WON % 2 == 0 and FA % FR == 0 and (F - FA) % FR == 0 and FA >= F - FA
    assert CPG >= NHG + 1

    def kernel(x_hbm, k_hbm, v_hbm, wq_hbm, wo_hbm, w1_hbm, b1_hbm, w2_hbm, b2_hbm, c_hbm, wm_hbm,
               out_ref,
               x_v, c_v, b1_v, b2_v, wm_v, wq_v, wo_v, w1_v, w2_v, kbuf, vbuf,
               q_scr, s_scr, p_scr, o_scr, mod_scr,
               sem_s, sem_w, sem_k, sem_v):
        _st = []

        def mark(name):
            if not scopes:
                return
            if _st:
                _st.pop().__exit__(None, None, None)
            if name:
                cm = jax.named_scope(name)
                cm.__enter__()
                _st.append(cm)

        small = [pltpu.make_async_copy(x_hbm, x_v, sem_s.at[0]),
                 pltpu.make_async_copy(c_hbm, c_v, sem_s.at[1]),
                 pltpu.make_async_copy(b1_hbm, b1_v, sem_s.at[2]),
                 pltpu.make_async_copy(b2_hbm, b2_v, sem_s.at[3])]

        def wait_region(ref, sem):
            pltpu.make_async_copy(ref, ref, sem).wait()

        def kv_copy(hbm, buf, sem, u, slot, d):
            g = u // CPG
            cj = u % CPG
            hg = g // B
            b = g % B
            r0 = pl.multiple_of(OFF + cj * R + d * DR, DR)
            return pltpu.make_async_copy(
                hbm.at[b, pl.ds(hg * GH, GH), pl.ds(r0, DR), :],
                buf.at[slot, :, pl.ds(d * DR if isinstance(d, int) else pl.multiple_of(d * DR, DR), DR), :],
                sem.at[slot])

        def k_copy(i):
            u = i // DPC
            return kv_copy(k_hbm, kbuf, sem_k, u, u % NK, i % DPC)

        def v_copy(i):
            u = i // DPC
            return kv_copy(v_hbm, vbuf, sem_v, u, u % NV, i % DPC)

        def wo_copy(i, odd):
            k = 2 * (i % (WON // 2)) + odd
            r0 = pl.multiple_of(k * (H * Dh // WON) + (i // (WON // 2)) * WOR, 8)
            return pltpu.make_async_copy(wo_hbm.at[pl.ds(r0, WOR), :], wo_v.at[pl.ds(r0, WOR), :],
                                         sem_w.at[SEM_WO])

        def issue_pairs(f0, f1, lo, hi):
            def step(p, _):
                f0(p).start(priority=1 - KP)
                f1(p).start(priority=KP)
                return 0
            lax.fori_loop(lo, hi, step, 0)

        def issue_kv(u):
            for d in range(DPC):
                du, dv = divmod(d - SH, DPC)
                kv_copy(v_hbm, vbuf, sem_v, u + du, (u + du) % NV, dv).start(priority=1 - KP)
                kv_copy(k_hbm, kbuf, sem_k, u, u % NK, d).start(priority=KP)

        SEM_WM, SEM_WQ, SEM_WO, SEM_W1A, SEM_W1B, SEM_W2A, SEM_W2B = range(7)

        mark('A_head_issue')
        if diag >= 3:
            class _N:
                def start(self): pass
                def wait(self): pass
            for cp in small: cp._used = True
            small = [_N()] * 4
        for cp in small:
            cp.start()
        TR = 8
        nrt = D // TR

        def head_step(t, _):
            for j in range(2):
                for k in range(HN):
                    r0 = pl.multiple_of((k * (nrt // HN) + t) * TR, TR)
                    for prio, (hbm, buf, sem) in enumerate(((wm_hbm, wm_v, sem_w.at[SEM_WM]),
                                                            (wq_hbm, wq_v, sem_w.at[SEM_WQ]))):
                        cw = buf.shape[1] // 2
                        sl = (pl.ds(r0, TR), pl.ds(j * cw, cw))
                        pltpu.make_async_copy(hbm.at[sl], buf.at[sl], sem).start(priority=prio)
            return 0

        lax.fori_loop(0, nrt // HN, head_step, 0)

        def issue_kv_range(u0, u1):
            def step(u, _):
                issue_kv(u)
                return 0
            if u1 > u0:
                lax.fori_loop(u0, u1, step, 0)

        issue_pairs(lambda p: wo_copy(p, 0), k_copy, 0, SH)
        issue_pairs(lambda p: v_copy(p - SH), k_copy, SH, 2 * DPC)

        mark('B_mod')
        small[0].wait()
        small[1].wait()
        x = x_v[...].astype(F32)
        sc = jax.nn.silu(c_v[...].astype(F32)).astype(BF16)
        wait_region(wm_v, sem_w.at[SEM_WM])
        mod_a = jnp.dot(sc, wm_v[:, 0:2 * D], preferred_element_type=F32)
        h = (_layernorm(x) * (1.0 + mod_a[:, D:2 * D]) + mod_a[:, 0:D]).astype(BF16)
        mark('C_issue')
        issue_kv_range(2, LA)

        def q_proj(hg):
            qq = jnp.dot(h, wq_v[:, hg * GH * Dh:(hg + 1) * GH * Dh], preferred_element_type=F32)
            qq = qq.astype(BF16).astype(F32)
            for j in range(GH):
                q_scr[pl.ds(hg * B * GH + j, B, stride=GH), :] = qq[:, j * Dh:(j + 1) * Dh]

        mark('D_q')
        wait_region(wq_v, sem_w.at[SEM_WQ])
        q_proj(0)

        row = lax.broadcasted_iota(jnp.int32, (GH, Dh), 0)

        def qk(u, g, cj):
            slot = u % NK
            wait_region(kbuf.at[slot], sem_k.at[slot])
            qg = q_scr[pl.ds(pl.multiple_of(g * GH, GH), GH), :]
            s = None
            for j in range(GH if compute else 1):
                qm = jnp.where(row == j, qg, 0.0).astype(BF16)
                t = lax.dot_general(qm, kbuf[slot, j], _NT, preferred_element_type=F32)
                s = t if s is None else s + t
            s_scr[cj] = s

        def pv(u, cj, acc):
            slot = u % NV
            wait_region(vbuf.at[slot], sem_v.at[slot])
            p = p_scr[cj].astype(BF16)
            for j in range(GH if compute else 1):
                t = jnp.dot(p, vbuf[slot, j], preferred_element_type=F32)
                acc = acc + jnp.where(row == j, t, 0.0)
            return acc

        def softmax():
            s = s_scr[...] * scale
            m = jnp.max(jnp.max(s, axis=0), axis=-1, keepdims=True)
            p = jnp.exp(s - m[None])
            p_scr[...] = p
            return jnp.sum(jnp.sum(p, axis=0), axis=-1, keepdims=True)

        def issue_next(u):
            n = u + LA

            @pl.when(n < NU)
            def _():
                issue_kv(n)

            @pl.when(n >= NU)
            def _():
                lo = ((n - NU) * n_wo) // LA
                hi = ((n - NU + 1) * n_wo) // LA
                issue_pairs(lambda p: v_copy(ND - SH + p), lambda p: wo_copy(p, 1),
                            lo, jnp.minimum(hi, SH))
                issue_pairs(lambda p: wo_copy(p, 0), lambda p: wo_copy(p, 1),
                            jnp.maximum(lo, SH), hi)

        def first_unit(cj, _):
            issue_next(cj)
            qk(cj, 0, cj)
            for hg in range(1, NHG):
                pl.when(cj == hg - 1)(functools.partial(q_proj, hg))
            for i in range(2):
                @pl.when(cj == NHG - 1 + i)
                def _():
                    mod_scr[:, 2 * i * D:2 * (i + 1) * D] = jnp.dot(
                        sc, wm_v[:, 2 * (i + 1) * D:2 * (i + 2) * D], preferred_element_type=F32)
            return 0

        mark('E_first')
        lax.fori_loop(0, CPG, first_unit, 0)
        l0 = softmax()

        def group(g, l_prev):
            def unit(cj, acc):
                u = g * CPG + cj
                issue_next(u)
                qk(u, g, cj)
                return pv(u - CPG, cj, acc)

            acc = lax.fori_loop(0, CPG, unit, jnp.zeros((GH, Dh), F32))
            o_scr[pl.ds(pl.multiple_of((g - 1) * GH, GH), GH), :] = acc / l_prev
            return softmax()

        mark('F_main')
        l_last = lax.fori_loop(1, NG, group, l0)
        mark('G_pvtail')

        def row_copy(hbm, buf, r0, sem):
            if not isinstance(r0, int):
                r0 = pl.multiple_of(r0, 8)
            return pltpu.make_async_copy(hbm.at[pl.ds(r0, FR), :], buf.at[pl.ds(r0, FR), :], sem)

        def issue_f(hbm, buf, sem_a, sem_b, t0, t1):
            def step(t, _):
                row_copy(hbm, buf, t * FR, sem_a).start(priority=0)
                row_copy(hbm, buf, FA + t * FR, sem_b).start(priority=1)
                return 0
            lax.fori_loop(t0, t1, step, 0)

        def issue_f_rest(hbm, buf, sem_a):
            for r0 in range(F - FA, FA, FR):
                row_copy(hbm, buf, r0, sem_a).start(priority=0)

        nb = (F - FA) // FR
        acc = jnp.zeros((GH, Dh), F32)
        for cj in range(CPG):
            acc = pv(NU - CPG + cj, cj, acc)
            if cj == CPG // 2 - 1:
                issue_f(w1_hbm, w1_v, sem_w.at[SEM_W1A], sem_w.at[SEM_W1B], 0, nb // 2)
        o_scr[pl.ds((NG - 1) * GH, GH), :] = acc / l_last
        mark('H_issue')
        issue_f(w1_hbm, w1_v, sem_w.at[SEM_W1A], sem_w.at[SEM_W1B], nb // 2, nb)
        issue_f_rest(w1_hbm, w1_v, sem_w.at[SEM_W1A])
        lo = FA
        for p, hi in enumerate(W2B):
            issue_f(w2_hbm, w2_v, sem_w.at[SEM_W2A], sem_w.at[SEM_W2B + p],
                    (lo - FA) // FR, (hi - FA) // FR)
            lo = hi
        issue_f_rest(w2_hbm, w2_v, sem_w.at[SEM_W2A])

        mark('I_waitwo')
        wait_region(wo_v, sem_w.at[SEM_WO])
        mark('J_wo')
        attn = None
        for hg in range(NHG):
            o = jnp.concatenate(
                [o_scr[pl.ds(hg * B * GH + j, B, stride=GH), :] for j in range(GH)], axis=1)
            t = jnp.dot(o.astype(BF16), wo_v[hg * GH * Dh:(hg + 1) * GH * Dh, :],
                        preferred_element_type=F32)
            attn = t if attn is None else attn + t

        ga, sb, cb, gb = (mod_scr[:, i * D:(i + 1) * D] for i in range(4))
        x1 = x + ga * attn
        h2 = (_layernorm(x1) * (1.0 + cb) + sb).astype(BF16)
        small[2].wait()
        small[3].wait()
        b1 = b1_v[...].astype(F32).reshape(1, F)
        b2 = b2_v[...].astype(F32).reshape(1, D)
        f1 = []
        for sem, lo, hi in ((SEM_W1A, 0, FA), (SEM_W1B, FA, F)):
            mark('K_waitw1_%d' % lo)
            wait_region(w1_v.at[pl.ds(lo, hi - lo), :], sem_w.at[sem])
            mark('L_ffn1_%d' % lo)
            t = lax.dot_general(h2, w1_v[lo:hi, :], _NT, preferred_element_type=F32) + b1[:, lo:hi]
            f1.append(jax.nn.gelu(t, approximate=True).astype(BF16))

        bounds = (FA,) + tuple(W2B)
        parts = [(SEM_W2A, 0, FA, f1[0])]
        for p in range(len(W2B)):
            lo, hi = bounds[p], bounds[p + 1]
            parts.append((SEM_W2B + p, lo, hi, f1[1][:, lo - FA:hi - FA]))
        y = b2
        for sem, lo, hi, f in parts:
            mark('M_waitw2_%d' % lo)
            wait_region(w2_v.at[pl.ds(lo, hi - lo), :], sem_w.at[sem])
            mark('N_ffn2_%d' % lo)
            if diag == 2 or (diag == 1 and hi == F):
                continue
            y = y + jnp.dot(f, w2_v[lo:hi, :], preferred_element_type=F32)
        if diag >= 4:
            out_ref[...] = jnp.zeros(out_ref.shape, out_ref.dtype)
        else:
            out_ref[...] = (x1 + gb * y).astype(out_ref.dtype)
        mark(None)

    scratch = [
        pltpu.VMEM((B, D), BF16), pltpu.VMEM((B, D), BF16),
        pltpu.VMEM((F,), BF16), pltpu.VMEM((D,), BF16),
        pltpu.VMEM((D, 6 * D), BF16), pltpu.VMEM((D, H * Dh), BF16),
        pltpu.VMEM((H * Dh, D), BF16), pltpu.VMEM((F, D), BF16), pltpu.VMEM((F, D), BF16),
        pltpu.VMEM((NK, GH, R, Dh), BF16), pltpu.VMEM((NV, GH, R, Dh), BF16),
        pltpu.VMEM((NG * GH, Dh), F32), pltpu.VMEM((CPG, GH, R), F32),
        pltpu.VMEM((CPG, GH, R), F32), pltpu.VMEM((NG * GH, Dh), F32), pltpu.VMEM((B, 4 * D), F32),
        pltpu.SemaphoreType.DMA((4,)), pltpu.SemaphoreType.DMA((6 + len(W2B),)),
        pltpu.SemaphoreType.DMA((NK,)), pltpu.SemaphoreType.DMA((NV,)),
    ]
    return kernel, scratch


@jax.jit
def pallas_adaLN_cond__sliding_block_cached__dense_activation_gelu__decode_kernel(
    A_x: jax.Array,
    A_k_cache: jax.Array,
    A_v_cache: jax.Array,
    A_wq: jax.Array,
    A_wo: jax.Array,
    B_x: jax.Array,
    B_w1: jax.Array,
    B_b1: jax.Array,
    B_w2: jax.Array,
    B_b2: jax.Array,
    c: jax.Array,
    w_mod: jax.Array,
):
    B, _, D = A_x.shape
    _, H, Sk, Dh = A_k_cache.shape
    F = B_w1.shape[1]
    kernel, scratch = _build(B, D, H, Sk, Dh, F, R=256, LA=6, NK=8, NV=16, SH=26)
    out = pl.pallas_call(
        kernel,
        in_specs=[pl.BlockSpec(memory_space=pl.ANY)] * 11,
        out_specs=pl.BlockSpec(memory_space=pltpu.VMEM),
        out_shape=jax.ShapeDtypeStruct((B, D), A_x.dtype),
        scratch_shapes=scratch,
        compiler_params=pltpu.CompilerParams(
            vmem_limit_bytes=100 * 1024 * 1024, disable_bounds_checks=True, disable_semaphore_checks=True),
    )(A_x.reshape(B, D), A_k_cache, A_v_cache, A_wq, A_wo, B_w1.T, B_b1, B_w2, B_b2, c, w_mod)
    return out.reshape(B, 1, D)
```

```python
import functools

import jax
import jax.numpy as jnp
from jax import lax
import jax.experimental.pallas as pl
import jax.experimental.pallas.tpu as pltpu

F32 = jnp.float32
BF16 = jnp.bfloat16

_NT = (((1,), (1,)), ((), ()))


def _layernorm(x, eps=1e-5):
    m = jnp.mean(x, axis=-1, keepdims=True)
    d = x - m
    v = jnp.mean(d * d, axis=-1, keepdims=True)
    return d * lax.rsqrt(v + eps)


def _build(B, D, H, Sk, Dh, F, *, R, LA, NS, SH, HN=4, WON=8, WOR=16, FR=32, FN=3,
           W2B=((1376, 4), (1632, 2), (1728, 1)), scopes=False):
    W = min(4096, max(256, Sk // 4))
    OFF = Sk - W
    GH = 8
    NHALF = H // (2 * GH)
    NSG = NHALF * B
    CPP = W // R
    NU = NSG * 2 * CPP
    DR = 16
    DPC = R // DR
    ND = NU * DPC
    TR = 8
    FA = F // 2
    n_wo = H * Dh // (2 * WOR)
    scale = float(Dh) ** -0.5
    SHU = -(-SH // DPC)
    assert LA >= SHU and NS > LA and SHU <= CPP and ((LA - SHU + 1) * n_wo) // LA >= SH
    assert FA % (FR * FN) == 0 and W2B[-1][0] == F and CPP >= 2 * (NHALF - 1) + 2

    SEM_WM, SEM_WQ, SEM_WO, SEM_W1A, SEM_W1B, SEM_W2A, SEM_W2B = range(7)

    def kernel(x_hbm, k_hbm, v_hbm, wq_hbm, wo_hbm, w1_hbm, b1_hbm, w2_hbm, b2_hbm, c_hbm, wm_hbm,
               out_ref,
               x_v, c_v, b1_v, b2_v, wm_v, wq_v, wo_v, w1_v, w2_v, kv_v,
               q_scr, s_scr, l_scr, acc_scr, o_scr, mod_scr,
               sem_s, sem_w, sem_kv):
        _st = []

        def mark(name):
            if not scopes:
                return
            if _st:
                _st.pop().__exit__(None, None, None)
            if name:
                cm = jax.named_scope(name)
                cm.__enter__()
                _st.append(cm)

        small = [pltpu.make_async_copy(x_hbm, x_v, sem_s.at[0]),
                 pltpu.make_async_copy(c_hbm, c_v, sem_s.at[1]),
                 pltpu.make_async_copy(b1_hbm, b1_v, sem_s.at[2]),
                 pltpu.make_async_copy(b2_hbm, b2_v, sem_s.at[3])]

        def wait_region(ref, sem):
            pltpu.make_async_copy(ref, ref, sem).wait()

        def is_v(u):
            return (u // CPP) % 2

        def kv_copy(hbm, th, u, d):
            sg = u // (2 * CPP)
            r0 = pl.multiple_of(OFF + (u % CPP) * R + d * DR, DR)
            d0 = d * DR if isinstance(d, int) else pl.multiple_of(d * DR, DR)
            return pltpu.make_async_copy(
                hbm.at[sg % B, sg // B, :, th, pl.ds(r0, DR), :],
                kv_v.at[th, u % NS, :, pl.ds(d0, DR), :],
                sem_kv.at[th, u % NS])

        def rows_copy(hbm, buf, sem, lo, hi, n, rows, i):
            assert (hi - lo) % (n * rows) == 0
            r0 = pl.multiple_of(lo + (i % n) * ((hi - lo) // n) + (i // n) * rows, TR)
            return pltpu.make_async_copy(hbm.at[pl.ds(r0, rows), :], buf.at[pl.ds(r0, rows), :], sem)

        def wo_copy(th, i):
            half = H * Dh // 2
            return rows_copy(wo_hbm, wo_v, sem_w.at[SEM_WO], th * half, (th + 1) * half,
                             WON // 2, WOR, i)

        def issue_pairs(f0, f1, lo, hi):
            def step(p, carry):
                f0(p).start(priority=0)
                f1(p).start(priority=1)
                return carry
            lax.fori_loop(lo, hi, step, 0)

        def issue_unit(u):
            runs = {}
            for d in range(DPC):
                du, d0 = divmod(d - SH, DPC)
                runs.setdefault(du, []).append((d, d0))
            for du, pairs in runs.items():
                for v1, hbm1 in enumerate((k_hbm, v_hbm)):
                    for v0, hbm0 in enumerate((k_hbm, v_hbm)):
                        @pl.when(jnp.logical_and(is_v(u) == v1, is_v(u + du) == v0))
                        def _(du=du, pairs=pairs, hbm0=hbm0, hbm1=hbm1):
                            for d, d0 in pairs:
                                kv_copy(hbm0, 0, u + du, d0).start(priority=0)
                                kv_copy(hbm1, 1, u, d).start(priority=1)

        mark('A_head_issue')
        for cp in small:
            cp.start()

        def head_step(t, carry):
            for j in range(2):
                for k in range(HN):
                    r0 = pl.multiple_of(k * (D // HN) + t * TR, TR)
                    for th, (hbm, buf, sem) in enumerate(((wm_hbm, wm_v, sem_w.at[SEM_WM]),
                                                          (wq_hbm, wq_v, sem_w.at[SEM_WQ]))):
                        cw = buf.shape[1] // 2
                        sl = (pl.ds(r0, TR), pl.ds(j * cw, cw))
                        pltpu.make_async_copy(hbm.at[sl], buf.at[sl], sem).start(priority=th)
            return carry

        lax.fori_loop(0, D // (HN * TR), head_step, 0)
        k1_copy = lambda p: kv_copy(k_hbm, 1, p // DPC, p % DPC)
        issue_pairs(functools.partial(wo_copy, 0), k1_copy, 0, SH)
        issue_pairs(lambda p: kv_copy(k_hbm, 0, (p - SH) // DPC, (p - SH) % DPC), k1_copy,
                    SH, SHU * DPC)

        mark('B_mod')
        small[0].wait()
        small[1].wait()
        x = x_v[...].astype(F32)
        sc = jax.nn.silu(c_v[...].astype(F32)).astype(BF16)
        wait_region(wm_v, sem_w.at[SEM_WM])
        mod_a = jnp.dot(sc, wm_v[:, 0:2 * D], preferred_element_type=F32)
        h = (_layernorm(x) * (1.0 + mod_a[:, D:2 * D]) + mod_a[:, 0:D]).astype(BF16)

        mark('C_issue')

        def prefill(u, carry):
            issue_unit(u)
            return carry

        lax.fori_loop(SHU, LA, prefill, 0)

        def head_rows(hd):
            half, r = divmod(hd, 2 * GH)
            j, th = divmod(r, 2)
            return pl.ds(half * B * 2 * GH + th * GH + j, B, stride=2 * GH)

        def q_proj(g):
            qq = jnp.dot(h, wq_v[:, g * GH * Dh:(g + 1) * GH * Dh], preferred_element_type=F32)
            qq = qq.astype(BF16).astype(F32)
            for j in range(GH):
                q_scr[head_rows(g * GH + j), :] = qq[:, j * Dh:(j + 1) * Dh]

        def mod_rest(i):
            mod_scr[:, 2 * i * D:2 * (i + 1) * D] = jnp.dot(
                sc, wm_v[:, 2 * (i + 1) * D:2 * (i + 2) * D], preferred_element_type=F32)

        mark('D_q')
        wait_region(wq_v, sem_w.at[SEM_WQ])
        q_proj(0)
        q_proj(1)
        acc_scr[...] = jnp.zeros(acc_scr.shape, F32)
        extras = [functools.partial(q_proj, g) for g in range(2, H // GH)]
        extras += [functools.partial(mod_rest, i) for i in range(2)]

        row = lax.broadcasted_iota(jnp.int32, (GH, Dh), 0)

        def unit(u, carry):
            n = u + LA

            @pl.when(n < NU)
            def _():
                issue_unit(n)

            @pl.when(n >= NU)
            def _():
                lo = ((n - NU) * n_wo) // LA
                hi = ((n - NU + 1) * n_wo) // LA
                issue_pairs(lambda p: kv_copy(v_hbm, 0, (ND - SH + p) // DPC, (ND - SH + p) % DPC),
                            functools.partial(wo_copy, 1), lo, jnp.minimum(hi, SH))
                issue_pairs(functools.partial(wo_copy, 0), functools.partial(wo_copy, 1),
                            jnp.maximum(lo, SH), hi)

            slot = u % NS
            cj = u % CPP
            sg = u // (2 * CPP)
            for th in range(2):
                wait_region(kv_v.at[th, slot], sem_kv.at[th, slot])

            @pl.when(is_v(u) == 0)
            def _():
                for th in range(2):
                    qg = q_scr[pl.ds(pl.multiple_of((2 * sg + th) * GH, GH), GH), :]
                    s = None
                    for j in range(GH):
                        qm = jnp.where(row == j, qg, 0.0).astype(BF16)
                        t = lax.dot_general(qm, kv_v[th, slot, j], _NT, preferred_element_type=F32)
                        s = t if s is None else s + t
                    s_scr[th, cj] = s

                @pl.when(cj == CPP - 1)
                def _():
                    for th in range(2):
                        s = s_scr[th] * scale
                        m = jnp.max(jnp.max(s, axis=0), axis=-1, keepdims=True)
                        p = jnp.exp(s - m[None])
                        s_scr[th] = p
                        l = jnp.sum(jnp.sum(p, axis=0), axis=-1, keepdims=True)
                        l_scr[th] = jnp.broadcast_to(l, (GH, Dh))

            @pl.when(is_v(u) == 1)
            def _():
                for th in range(2):
                    p = s_scr[th, cj].astype(BF16)
                    acc = acc_scr[th]
                    for j in range(GH):
                        t = jnp.dot(p, kv_v[th, slot, j], preferred_element_type=F32)
                        acc = acc + jnp.where(row == j, t, 0.0)
                    acc_scr[th] = acc

                @pl.when(cj == CPP - 1)
                def _():
                    for th in range(2):
                        o_scr[pl.ds(pl.multiple_of((2 * sg + th) * GH, GH), GH), :] = (
                            acc_scr[th] / l_scr[th])
                        acc_scr[th] = jnp.zeros((GH, Dh), F32)

            for i, extra in enumerate(extras):
                pl.when(u == i)(extra)
            return carry

        mark('F_main')
        lax.fori_loop(0, NU, unit, 0)

        mark('H_issue')
        nf = FA // FR
        issue_pairs(functools.partial(rows_copy, w1_hbm, w1_v, sem_w.at[SEM_W1A], 0, FA, FN, FR),
                    functools.partial(rows_copy, w1_hbm, w1_v, sem_w.at[SEM_W1B], FA, F, FN, FR),
                    0, nf)
        bounds = (FA,) + tuple(hi for hi, _ in W2B)
        for p, (hi, n) in enumerate(W2B):
            lo = bounds[p]
            t0 = (lo - FA) // FR
            issue_pairs(
                functools.partial(rows_copy, w2_hbm, w2_v, sem_w.at[SEM_W2A], 0, FA, FN, FR),
                lambda t, p=p, lo=lo, hi=hi, n=n, t0=t0: rows_copy(
                    w2_hbm, w2_v, sem_w.at[SEM_W2B + p], lo, hi, n, FR, t - t0),
                t0, (hi - FA) // FR)

        mark('I_waitwo')
        wait_region(wo_v, sem_w.at[SEM_WO])
        mark('J_wo')
        attn = None
        for g in range(H // GH):
            o = jnp.concatenate([o_scr[head_rows(g * GH + j), :] for j in range(GH)], axis=1)
            t = jnp.dot(o.astype(BF16), wo_v[g * GH * Dh:(g + 1) * GH * Dh, :],
                        preferred_element_type=F32)
            attn = t if attn is None else attn + t

        ga, sb, cb, gb = (mod_scr[:, i * D:(i + 1) * D] for i in range(4))
        x1 = x + ga * attn
        h2 = (_layernorm(x1) * (1.0 + cb) + sb).astype(BF16)
        small[2].wait()
        small[3].wait()
        b1 = b1_v[...].astype(F32).reshape(1, F)
        b2 = b2_v[...].astype(F32).reshape(1, D)
        f1 = []
        for sem, lo, hi in ((SEM_W1A, 0, FA), (SEM_W1B, FA, F)):
            mark('K_waitw1_%d' % lo)
            wait_region(w1_v.at[pl.ds(lo, hi - lo), :], sem_w.at[sem])
            mark('L_ffn1_%d' % lo)
            t = lax.dot_general(h2, w1_v[lo:hi, :], _NT, preferred_element_type=F32) + b1[:, lo:hi]
            f1.append(jax.nn.gelu(t, approximate=True).astype(BF16))

        parts = [(SEM_W2A, 0, FA, f1[0])]
        for p in range(len(W2B)):
            lo, hi = bounds[p], bounds[p + 1]
            parts.append((SEM_W2B + p, lo, hi, f1[1][:, lo - FA:hi - FA]))
        y = b2
        for sem, lo, hi, f in parts:
            mark('M_waitw2_%d' % lo)
            wait_region(w2_v.at[pl.ds(lo, hi - lo), :], sem_w.at[sem])
            mark('N_ffn2_%d' % lo)
            y = y + jnp.dot(f, w2_v[lo:hi, :], preferred_element_type=F32)
        out_ref[...] = (x1 + gb * y).astype(out_ref.dtype)
        mark(None)

    scratch = [
        pltpu.VMEM((B, D), BF16), pltpu.VMEM((B, D), BF16),
        pltpu.VMEM((F,), BF16), pltpu.VMEM((D,), BF16),
        pltpu.VMEM((D, 6 * D), BF16), pltpu.VMEM((D, H * Dh), BF16),
        pltpu.VMEM((H * Dh, D), BF16), pltpu.VMEM((F, D), BF16), pltpu.VMEM((F, D), BF16),
        pltpu.VMEM((2, NS, GH, R, Dh), BF16),
        pltpu.VMEM((B * H, Dh), F32), pltpu.VMEM((2, CPP, GH, R), F32),
        pltpu.VMEM((2, GH, Dh), F32), pltpu.VMEM((2, GH, Dh), F32),
        pltpu.VMEM((B * H, Dh), F32), pltpu.VMEM((B, 4 * D), F32),
        pltpu.SemaphoreType.DMA((4,)), pltpu.SemaphoreType.DMA((6 + len(W2B),)),
        pltpu.SemaphoreType.DMA((2, NS)),
    ]
    kv_shape = (B, NHALF, GH, 2, Sk, Dh)
    return kernel, scratch, kv_shape


@jax.jit
def pallas_adaLN_cond__sliding_block_cached__dense_activation_gelu__decode_kernel(
    A_x: jax.Array,
    A_k_cache: jax.Array,
    A_v_cache: jax.Array,
    A_wq: jax.Array,
    A_wo: jax.Array,
    B_x: jax.Array,
    B_w1: jax.Array,
    B_b1: jax.Array,
    B_w2: jax.Array,
    B_b2: jax.Array,
    c: jax.Array,
    w_mod: jax.Array,
):
    B, _, D = A_x.shape
    _, H, Sk, Dh = A_k_cache.shape
    F = B_w1.shape[1]
    kernel, scratch, kv_shape = _build(B, D, H, Sk, Dh, F, R=256, LA=6, NS=8, SH=26, W2B=((1248, 4), (1504, 4), (1728, 1)))
    out = pl.pallas_call(
        kernel,
        in_specs=[pl.BlockSpec(memory_space=pl.ANY)] * 11,
        out_specs=pl.BlockSpec(memory_space=pltpu.VMEM),
        out_shape=jax.ShapeDtypeStruct((B, D), A_x.dtype),
        scratch_shapes=scratch,
        compiler_params=pltpu.CompilerParams(
            vmem_limit_bytes=100 * 1024 * 1024, disable_bounds_checks=True,
            disable_semaphore_checks=True),
    )(A_x.reshape(B, D), A_k_cache.reshape(kv_shape), A_v_cache.reshape(kv_shape),
      A_wq, A_wo, B_w1.T, B_b1, B_w2, B_b2, c, w_mod)
    return out.reshape(B, 1, D)
```

```python
import functools

import jax
import jax.numpy as jnp
from jax import lax
import jax.experimental.pallas as pl
import jax.experimental.pallas.tpu as pltpu

F32 = jnp.float32
BF16 = jnp.bfloat16

_NT = (((1,), (1,)), ((), ()))


def _layernorm(x, eps=1e-5):
    m = jnp.mean(x, axis=-1, keepdims=True)
    d = x - m
    v = jnp.mean(d * d, axis=-1, keepdims=True)
    return d * lax.rsqrt(v + eps)


def _build(B, D, H, Sk, Dh, F, *, R, LA, NS, SH, HN=4, WON=8, WOR=16, FR=32, FN=3,
           W2B=((1376, 4), (1632, 2), (1728, 1))):
    W = min(4096, max(256, Sk // 4))
    OFF = Sk - W
    GH = 8
    NHALF = H // (2 * GH)
    NSG = NHALF * B
    CPP = W // R
    NU = NSG * 2 * CPP
    DR = 16
    DPC = R // DR
    ND = NU * DPC
    TR = 8
    FA = F // 2
    n_wo = H * Dh // (2 * WOR)
    scale = float(Dh) ** -0.5
    SHU = -(-SH // DPC)
    assert LA >= SHU and NS > LA and SHU <= CPP and ((LA - SHU + 1) * n_wo) // LA >= SH
    assert FA % (FR * FN) == 0 and W2B[-1][0] == F and CPP >= 2 * (NHALF - 1) + 2

    SEM_WM, SEM_WQ, SEM_WO, SEM_W1A, SEM_W1B, SEM_W2A, SEM_W2B = range(7)

    def kernel(x_hbm, k_hbm, v_hbm, wq_hbm, wo_hbm, w1_hbm, b1_hbm, w2_hbm, b2_hbm, c_hbm, wm_hbm,
               out_ref,
               x_v, c_v, b1_v, b2_v, wm_v, wq_v, wo_v, w1_v, w2_v, kv_v,
               q_scr, s_scr, l_scr, acc_scr, o_scr, mod_scr,
               sem_s, sem_w, sem_kv):
        small = [pltpu.make_async_copy(x_hbm, x_v, sem_s.at[0]),
                 pltpu.make_async_copy(c_hbm, c_v, sem_s.at[1]),
                 pltpu.make_async_copy(b1_hbm, b1_v, sem_s.at[2]),
                 pltpu.make_async_copy(b2_hbm, b2_v, sem_s.at[3])]

        def wait_region(ref, sem):
            pltpu.make_async_copy(ref, ref, sem).wait()

        def is_v(u):
            return (u // CPP) % 2

        def kv_copy(hbm, th, u, d):
            sg = u // (2 * CPP)
            r0 = pl.multiple_of(OFF + (u % CPP) * R + d * DR, DR)
            d0 = d * DR if isinstance(d, int) else pl.multiple_of(d * DR, DR)
            return pltpu.make_async_copy(
                hbm.at[sg % B, sg // B, :, th, pl.ds(r0, DR), :],
                kv_v.at[th, u % NS, :, pl.ds(d0, DR), :],
                sem_kv.at[th, u % NS])

        def rows_copy(hbm, buf, sem, lo, hi, n, rows, i):
            assert (hi - lo) % (n * rows) == 0
            r0 = pl.multiple_of(lo + (i % n) * ((hi - lo) // n) + (i // n) * rows, TR)
            return pltpu.make_async_copy(hbm.at[pl.ds(r0, rows), :], buf.at[pl.ds(r0, rows), :], sem)

        def wo_copy(th, i):
            half = H * Dh // 2
            return rows_copy(wo_hbm, wo_v, sem_w.at[SEM_WO], th * half, (th + 1) * half,
                             WON // 2, WOR, i)

        def issue_pairs(f0, f1, lo, hi):
            def step(p, carry):
                f0(p).start(priority=0)
                f1(p).start(priority=1)
                return carry
            lax.fori_loop(lo, hi, step, 0)

        def issue_unit(u):
            runs = {}
            for d in range(DPC):
                du, d0 = divmod(d - SH, DPC)
                runs.setdefault(du, []).append((d, d0))
            for du, pairs in runs.items():
                for v1, hbm1 in enumerate((k_hbm, v_hbm)):
                    for v0, hbm0 in enumerate((k_hbm, v_hbm)):
                        @pl.when(jnp.logical_and(is_v(u) == v1, is_v(u + du) == v0))
                        def _(du=du, pairs=pairs, hbm0=hbm0, hbm1=hbm1):
                            for d, d0 in pairs:
                                kv_copy(hbm0, 0, u + du, d0).start(priority=0)
                                kv_copy(hbm1, 1, u, d).start(priority=1)

        for cp in small:
            cp.start()

        def head_step(t, carry):
            for j in range(2):
                for k in range(HN):
                    r0 = pl.multiple_of(k * (D // HN) + t * TR, TR)
                    for th, (hbm, buf, sem) in enumerate(((wm_hbm, wm_v, sem_w.at[SEM_WM]),
                                                          (wq_hbm, wq_v, sem_w.at[SEM_WQ]))):
                        cw = buf.shape[1] // 2
                        sl = (pl.ds(r0, TR), pl.ds(j * cw, cw))
                        pltpu.make_async_copy(hbm.at[sl], buf.at[sl], sem).start(priority=th)
            return carry

        lax.fori_loop(0, D // (HN * TR), head_step, 0)
        k1_copy = lambda p: kv_copy(k_hbm, 1, p // DPC, p % DPC)
        issue_pairs(functools.partial(wo_copy, 0), k1_copy, 0, SH)
        issue_pairs(lambda p: kv_copy(k_hbm, 0, (p - SH) // DPC, (p - SH) % DPC), k1_copy,
                    SH, SHU * DPC)

        small[0].wait()
        small[1].wait()
        x = x_v[...].astype(F32)
        sc = jax.nn.silu(c_v[...].astype(F32)).astype(BF16)
        wait_region(wm_v, sem_w.at[SEM_WM])
        mod_a = jnp.dot(sc, wm_v[:, 0:2 * D], preferred_element_type=F32)
        h = (_layernorm(x) * (1.0 + mod_a[:, D:2 * D]) + mod_a[:, 0:D]).astype(BF16)


        def prefill(u, carry):
            issue_unit(u)
            return carry

        lax.fori_loop(SHU, LA, prefill, 0)

        def head_rows(hd):
            half, r = divmod(hd, 2 * GH)
            j, th = divmod(r, 2)
            return pl.ds(half * B * 2 * GH + th * GH + j, B, stride=2 * GH)

        def q_proj(g):
            qq = jnp.dot(h, wq_v[:, g * GH * Dh:(g + 1) * GH * Dh], preferred_element_type=F32)
            qq = qq.astype(BF16).astype(F32)
            for j in range(GH):
                q_scr[head_rows(g * GH + j), :] = qq[:, j * Dh:(j + 1) * Dh]

        def mod_rest(i):
            mod_scr[:, 2 * i * D:2 * (i + 1) * D] = jnp.dot(
                sc, wm_v[:, 2 * (i + 1) * D:2 * (i + 2) * D], preferred_element_type=F32)

        wait_region(wq_v, sem_w.at[SEM_WQ])
        q_proj(0)
        q_proj(1)
        acc_scr[...] = jnp.zeros(acc_scr.shape, F32)
        extras = [functools.partial(q_proj, g) for g in range(2, H // GH)]
        extras += [functools.partial(mod_rest, i) for i in range(2)]

        row = lax.broadcasted_iota(jnp.int32, (GH, Dh), 0)

        def unit(u, carry):
            n = u + LA

            @pl.when(n < NU)
            def _():
                issue_unit(n)

            @pl.when(n >= NU)
            def _():
                lo = ((n - NU) * n_wo) // LA
                hi = ((n - NU + 1) * n_wo) // LA
                issue_pairs(lambda p: kv_copy(v_hbm, 0, (ND - SH + p) // DPC, (ND - SH + p) % DPC),
                            functools.partial(wo_copy, 1), lo, jnp.minimum(hi, SH))
                issue_pairs(functools.partial(wo_copy, 0), functools.partial(wo_copy, 1),
                            jnp.maximum(lo, SH), hi)

            slot = u % NS
            cj = u % CPP
            sg = u // (2 * CPP)
            for th in range(2):
                wait_region(kv_v.at[th, slot], sem_kv.at[th, slot])

            @pl.when(is_v(u) == 0)
            def _():
                for th in range(2):
                    qg = q_scr[pl.ds(pl.multiple_of((2 * sg + th) * GH, GH), GH), :]
                    s = None
                    for j in range(GH):
                        qm = jnp.where(row == j, qg, 0.0).astype(BF16)
                        t = lax.dot_general(qm, kv_v[th, slot, j], _NT, preferred_element_type=F32)
                        s = t if s is None else s + t
                    s_scr[th, cj] = s

                @pl.when(cj == CPP - 1)
                def _():
                    for th in range(2):
                        s = s_scr[th] * scale
                        m = jnp.max(jnp.max(s, axis=0), axis=-1, keepdims=True)
                        p = jnp.exp(s - m[None])
                        s_scr[th] = p
                        l = jnp.sum(jnp.sum(p, axis=0), axis=-1, keepdims=True)
                        l_scr[th] = jnp.broadcast_to(l, (GH, Dh))

            @pl.when(is_v(u) == 1)
            def _():
                for th in range(2):
                    p = s_scr[th, cj].astype(BF16)
                    acc = acc_scr[th]
                    for j in range(GH):
                        t = jnp.dot(p, kv_v[th, slot, j], preferred_element_type=F32)
                        acc = acc + jnp.where(row == j, t, 0.0)
                    acc_scr[th] = acc

                @pl.when(cj == CPP - 1)
                def _():
                    for th in range(2):
                        o_scr[pl.ds(pl.multiple_of((2 * sg + th) * GH, GH), GH), :] = (
                            acc_scr[th] / l_scr[th])
                        acc_scr[th] = jnp.zeros((GH, Dh), F32)

            for i, extra in enumerate(extras):
                pl.when(u == i)(extra)
            return carry

        lax.fori_loop(0, NU, unit, 0)

        nf = FA // FR
        issue_pairs(functools.partial(rows_copy, w1_hbm, w1_v, sem_w.at[SEM_W1A], 0, FA, FN, FR),
                    functools.partial(rows_copy, w1_hbm, w1_v, sem_w.at[SEM_W1B], FA, F, FN, FR),
                    0, nf)
        bounds = (FA,) + tuple(hi for hi, _ in W2B)
        for p, (hi, n) in enumerate(W2B):
            lo = bounds[p]
            t0 = (lo - FA) // FR
            issue_pairs(
                functools.partial(rows_copy, w2_hbm, w2_v, sem_w.at[SEM_W2A], 0, FA, FN, FR),
                lambda t, p=p, lo=lo, hi=hi, n=n, t0=t0: rows_copy(
                    w2_hbm, w2_v, sem_w.at[SEM_W2B + p], lo, hi, n, FR, t - t0),
                t0, (hi - FA) // FR)

        wait_region(wo_v, sem_w.at[SEM_WO])
        attn = None
        for g in range(H // GH):
            o = jnp.concatenate([o_scr[head_rows(g * GH + j), :] for j in range(GH)], axis=1)
            t = jnp.dot(o.astype(BF16), wo_v[g * GH * Dh:(g + 1) * GH * Dh, :],
                        preferred_element_type=F32)
            attn = t if attn is None else attn + t

        ga, sb, cb, gb = (mod_scr[:, i * D:(i + 1) * D] for i in range(4))
        x1 = x + ga * attn
        h2 = (_layernorm(x1) * (1.0 + cb) + sb).astype(BF16)
        small[2].wait()
        small[3].wait()
        b1 = b1_v[...].astype(F32).reshape(1, F)
        b2 = b2_v[...].astype(F32).reshape(1, D)
        f1 = []
        for sem, lo, hi in ((SEM_W1A, 0, FA), (SEM_W1B, FA, F)):
            wait_region(w1_v.at[pl.ds(lo, hi - lo), :], sem_w.at[sem])
            t = lax.dot_general(h2, w1_v[lo:hi, :], _NT, preferred_element_type=F32) + b1[:, lo:hi]
            f1.append(jax.nn.gelu(t, approximate=True).astype(BF16))

        parts = [(SEM_W2A, 0, FA, f1[0])]
        for p in range(len(W2B)):
            lo, hi = bounds[p], bounds[p + 1]
            parts.append((SEM_W2B + p, lo, hi, f1[1][:, lo - FA:hi - FA]))
        y = b2
        for sem, lo, hi, f in parts:
            wait_region(w2_v.at[pl.ds(lo, hi - lo), :], sem_w.at[sem])
            y = y + jnp.dot(f, w2_v[lo:hi, :], preferred_element_type=F32)
        out_ref[...] = (x1 + gb * y).astype(out_ref.dtype)

    scratch = [
        pltpu.VMEM((B, D), BF16), pltpu.VMEM((B, D), BF16),
        pltpu.VMEM((F,), BF16), pltpu.VMEM((D,), BF16),
        pltpu.VMEM((D, 6 * D), BF16), pltpu.VMEM((D, H * Dh), BF16),
        pltpu.VMEM((H * Dh, D), BF16), pltpu.VMEM((F, D), BF16), pltpu.VMEM((F, D), BF16),
        pltpu.VMEM((2, NS, GH, R, Dh), BF16),
        pltpu.VMEM((B * H, Dh), F32), pltpu.VMEM((2, CPP, GH, R), F32),
        pltpu.VMEM((2, GH, Dh), F32), pltpu.VMEM((2, GH, Dh), F32),
        pltpu.VMEM((B * H, Dh), F32), pltpu.VMEM((B, 4 * D), F32),
        pltpu.SemaphoreType.DMA((4,)), pltpu.SemaphoreType.DMA((6 + len(W2B),)),
        pltpu.SemaphoreType.DMA((2, NS)),
    ]
    kv_shape = (B, NHALF, GH, 2, Sk, Dh)
    return kernel, scratch, kv_shape


@jax.jit
def pallas_adaLN_cond__sliding_block_cached__dense_activation_gelu__decode_kernel(
    A_x: jax.Array,
    A_k_cache: jax.Array,
    A_v_cache: jax.Array,
    A_wq: jax.Array,
    A_wo: jax.Array,
    B_x: jax.Array,
    B_w1: jax.Array,
    B_b1: jax.Array,
    B_w2: jax.Array,
    B_b2: jax.Array,
    c: jax.Array,
    w_mod: jax.Array,
):
    B, _, D = A_x.shape
    _, H, Sk, Dh = A_k_cache.shape
    F = B_w1.shape[1]
    kernel, scratch, kv_shape = _build(B, D, H, Sk, Dh, F, R=256, LA=6, NS=8, SH=26)
    out = pl.pallas_call(
        kernel,
        in_specs=[pl.BlockSpec(memory_space=pl.ANY)] * 11,
        out_specs=pl.BlockSpec(memory_space=pltpu.VMEM),
        out_shape=jax.ShapeDtypeStruct((B, D), A_x.dtype),
        scratch_shapes=scratch,
        compiler_params=pltpu.CompilerParams(
            vmem_limit_bytes=64 * 1024 * 1024, disable_bounds_checks=True,
            disable_semaphore_checks=True),
    )(A_x.reshape(B, D), A_k_cache.reshape(kv_shape), A_v_cache.reshape(kv_shape),
      A_wq, A_wo, B_w1.T, B_b1, B_w2, B_b2, c, w_mod)
    return out.reshape(B, 1, D)
```

```python
import functools

import jax
import jax.numpy as jnp
from jax import lax
import jax.experimental.pallas as pl
import jax.experimental.pallas.tpu as pltpu

F32 = jnp.float32
BF16 = jnp.bfloat16

_NT = (((1,), (1,)), ((), ()))


def _layernorm(x, eps=1e-5):
    m = jnp.mean(x, axis=-1, keepdims=True)
    d = x - m
    v = jnp.mean(d * d, axis=-1, keepdims=True)
    return d * lax.rsqrt(v + eps)


def _build(B, D, H, Sk, Dh, F, *, R, LA, NS, SH, HN=4, WON=8, WOR=16, FR=32, FN=3,
           W2B=((384, 4), (640, 4)), VG=(6, 4, 3, 1), VR=16):
    W = min(4096, max(256, Sk // 4))
    OFF = Sk - W
    GH = 8
    NHALF = H // (2 * GH)
    NSG = NHALF * B
    CPP = W // R
    NU = NSG * 2 * CPP
    DR = 16
    DPC = R // DR
    ND = NU * DPC
    TR = 8
    FA = F // 2
    n_wo = H * Dh // (2 * WOR)
    scale = float(Dh) ** -0.5
    SHU = -(-SH // DPC)
    assert LA >= SHU and NS > LA and SHU <= CPP and ((LA - SHU + 1) * n_wo) // LA >= SH
    VLO = W2B[-1][0]
    assert FA % (FR * FN) == 0 and VLO + sum(VG) * VR == FA and VLO % 128 == 0

    SEM_WM, SEM_WQ, SEM_WO, SEM_W1A, SEM_W1B, SEM_W2A, SEM_W2B = range(7)

    def kernel(x_hbm, k_hbm, v_hbm, wq_hbm, wo_hbm, w1_hbm, b1_hbm, w2_hbm, b2_hbm, c_hbm, wm_hbm,
               out_ref,
               x_v, c_v, b1_v, b2_v, wm_v, wq_v, wo_v, w1_v, w2_v, kv_v,
               q_scr, s_scr, l_scr, acc_scr, o_scr, mod_scr, fb_scr,
               sem_s, sem_w, sem_kv):
        small = [pltpu.make_async_copy(x_hbm, x_v, sem_s.at[0]),
                 pltpu.make_async_copy(c_hbm, c_v, sem_s.at[1]),
                 pltpu.make_async_copy(b1_hbm, b1_v, sem_s.at[2]),
                 pltpu.make_async_copy(b2_hbm, b2_v, sem_s.at[3])]

        def wait_region(ref, sem):
            pltpu.make_async_copy(ref, ref, sem).wait()

        def is_v(u):
            return (u // CPP) % 2

        def kv_copy(hbm, th, u, d):
            sg = u // (2 * CPP)
            r0 = pl.multiple_of(OFF + (u % CPP) * R + d * DR, DR)
            d0 = d * DR if isinstance(d, int) else pl.multiple_of(d * DR, DR)
            return pltpu.make_async_copy(
                hbm.at[sg % B, sg // B, :, th, pl.ds(r0, DR), :],
                kv_v.at[th, u % NS, :, pl.ds(d0, DR), :],
                sem_kv.at[th, u % NS])

        def rows_copy(hbm, buf, sem, lo, hi, n, rows, i):
            assert (hi - lo) % (n * rows) == 0
            r0 = pl.multiple_of(lo + (i % n) * ((hi - lo) // n) + (i // n) * rows, TR)
            return pltpu.make_async_copy(hbm.at[pl.ds(r0, rows), :], buf.at[pl.ds(r0, rows), :], sem)

        def wo_copy(th, i):
            half = H * Dh // 2
            return rows_copy(wo_hbm, wo_v, sem_w.at[SEM_WO], th * half, (th + 1) * half,
                             WON // 2, WOR, i)

        def issue_pairs(f0, f1, lo, hi):
            def step(p, carry):
                f0(p).start(priority=0)
                f1(p).start(priority=1)
                return carry
            lax.fori_loop(lo, hi, step, 0)

        def issue_unit(u):
            runs = {}
            for d in range(DPC):
                du, d0 = divmod(d - SH, DPC)
                runs.setdefault(du, []).append((d, d0))
            for du, pairs in runs.items():
                for v1, hbm1 in enumerate((k_hbm, v_hbm)):
                    for v0, hbm0 in enumerate((k_hbm, v_hbm)):
                        @pl.when(jnp.logical_and(is_v(u) == v1, is_v(u + du) == v0))
                        def _(du=du, pairs=pairs, hbm0=hbm0, hbm1=hbm1):
                            for d, d0 in pairs:
                                kv_copy(hbm0, 0, u + du, d0).start(priority=0)
                                kv_copy(hbm1, 1, u, d).start(priority=1)

        for cp in small:
            cp.start()

        def head_step(t, carry):
            for j in range(2):
                for k in range(HN):
                    r0 = pl.multiple_of(k * (D // HN) + t * TR, TR)
                    for th, (hbm, buf, sem) in enumerate(((wm_hbm, wm_v, sem_w.at[SEM_WM]),
                                                          (wq_hbm, wq_v, sem_w.at[SEM_WQ]))):
                        cw = buf.shape[1] // 2
                        sl = (pl.ds(r0, TR), pl.ds(j * cw, cw))
                        pltpu.make_async_copy(hbm.at[sl], buf.at[sl], sem).start(priority=th)
            return carry

        lax.fori_loop(0, D // (HN * TR), head_step, 0)
        k1_copy = lambda p: kv_copy(k_hbm, 1, p // DPC, p % DPC)
        issue_pairs(functools.partial(wo_copy, 0), k1_copy, 0, SH)
        issue_pairs(lambda p: kv_copy(k_hbm, 0, (p - SH) // DPC, (p - SH) % DPC), k1_copy,
                    SH, SHU * DPC)

        small[0].wait()
        small[1].wait()
        x = x_v[...].astype(F32)
        sc = jax.nn.silu(c_v[...].astype(F32)).astype(BF16)
        wait_region(wm_v, sem_w.at[SEM_WM])
        mod_a = jnp.dot(sc, wm_v[:, 0:2 * D], preferred_element_type=F32)
        h = (_layernorm(x) * (1.0 + mod_a[:, D:2 * D]) + mod_a[:, 0:D]).astype(BF16)

        def prefill(u, carry):
            issue_unit(u)
            return carry

        lax.fori_loop(SHU, LA, prefill, 0)

        def head_rows(hd):
            half, r = divmod(hd, 2 * GH)
            j, th = divmod(r, 2)
            return pl.ds(half * B * 2 * GH + th * GH + j, B, stride=2 * GH)

        def q_proj(g):
            qq = jnp.dot(h, wq_v[:, g * GH * Dh:(g + 1) * GH * Dh], preferred_element_type=F32)
            qq = qq.astype(BF16).astype(F32)
            for j in range(GH):
                q_scr[head_rows(g * GH + j), :] = qq[:, j * Dh:(j + 1) * Dh]

        def mod_rest(i):
            mod_scr[:, 2 * i * D:2 * (i + 1) * D] = jnp.dot(
                sc, wm_v[:, 2 * (i + 1) * D:2 * (i + 2) * D], preferred_element_type=F32)

        wait_region(wq_v, sem_w.at[SEM_WQ])
        q_proj(0)
        q_proj(1)
        acc_scr[...] = jnp.zeros(acc_scr.shape, F32)
        extras = [functools.partial(q_proj, g) for g in range(2, H // GH)]
        extras += [functools.partial(mod_rest, i) for i in range(2)]

        row = lax.broadcasted_iota(jnp.int32, (GH, Dh), 0)

        def unit(u, carry):
            n = u + LA

            @pl.when(n < NU)
            def _():
                issue_unit(n)

            @pl.when(n >= NU)
            def _():
                lo = ((n - NU) * n_wo) // LA
                hi = ((n - NU + 1) * n_wo) // LA
                issue_pairs(lambda p: kv_copy(v_hbm, 0, (ND - SH + p) // DPC, (ND - SH + p) % DPC),
                            functools.partial(wo_copy, 1), lo, jnp.minimum(hi, SH))
                issue_pairs(functools.partial(wo_copy, 0), functools.partial(wo_copy, 1),
                            jnp.maximum(lo, SH), hi)

            slot = u % NS
            cj = u % CPP
            sg = u // (2 * CPP)
            for th in range(2):
                wait_region(kv_v.at[th, slot], sem_kv.at[th, slot])

            @pl.when(is_v(u) == 0)
            def _():
                for th in range(2):
                    qg = q_scr[pl.ds(pl.multiple_of((2 * sg + th) * GH, GH), GH), :]
                    s = None
                    for j in range(GH):
                        qm = jnp.where(row == j, qg, 0.0).astype(BF16)
                        t = lax.dot_general(qm, kv_v[th, slot, j], _NT, preferred_element_type=F32)
                        s = t if s is None else s + t
                    s_scr[th, cj] = s

                @pl.when(cj == CPP - 1)
                def _():
                    for th in range(2):
                        s = s_scr[th] * scale
                        m = jnp.max(jnp.max(s, axis=0), axis=-1, keepdims=True)
                        p = jnp.exp(s - m[None])
                        s_scr[th] = p
                        l = jnp.sum(jnp.sum(p, axis=0), axis=-1, keepdims=True)
                        l_scr[th] = jnp.broadcast_to(l, (GH, Dh))

            @pl.when(is_v(u) == 1)
            def _():
                for th in range(2):
                    p = s_scr[th, cj].astype(BF16)
                    acc = acc_scr[th]
                    for j in range(GH):
                        t = jnp.dot(p, kv_v[th, slot, j], preferred_element_type=F32)
                        acc = acc + jnp.where(row == j, t, 0.0)
                    acc_scr[th] = acc

                @pl.when(cj == CPP - 1)
                def _():
                    for th in range(2):
                        o_scr[pl.ds(pl.multiple_of((2 * sg + th) * GH, GH), GH), :] = (
                            acc_scr[th] / l_scr[th])
                        acc_scr[th] = jnp.zeros((GH, Dh), F32)

            for i, extra in enumerate(extras):
                pl.when(u == i)(extra)
            return carry

        lax.fori_loop(0, NU, unit, 0)

        nf = FA // FR
        issue_pairs(functools.partial(rows_copy, w1_hbm, w1_v, sem_w.at[SEM_W1A], 0, FA, FN, FR),
                    functools.partial(rows_copy, w1_hbm, w1_v, sem_w.at[SEM_W1B], FA, F, FN, FR),
                    0, nf)
        bounds = (0,) + tuple(hi for hi, _ in W2B)
        for p, (hi, n) in enumerate(W2B):
            lo = bounds[p]
            t0 = lo // FR
            issue_pairs(
                functools.partial(rows_copy, w2_hbm, w2_v, sem_w.at[SEM_W2A], FA, F, FN, FR),
                lambda t, p=p, lo=lo, hi=hi, n=n, t0=t0: rows_copy(
                    w2_hbm, w2_v, sem_w.at[SEM_W2B + p], lo, hi, n, FR, t - t0),
                t0, hi // FR)

        SEM_V = SEM_W2B + len(W2B)
        v_starts = [sum(VG[:g]) for g in range(len(VG) + 1)]

        def v_copy(i):
            g = sum((i >= st).astype(jnp.int32) for st in v_starts[1:-1])
            r0 = pl.multiple_of(VLO + i * VR, TR)
            return pltpu.make_async_copy(w2_hbm.at[pl.ds(r0, VR), :], w2_v.at[pl.ds(r0, VR), :],
                                         sem_w.at[SEM_V + g])

        t0 = VLO // FR
        issue_pairs(lambda i: rows_copy(w2_hbm, w2_v, sem_w.at[SEM_W2A], FA, F, FN, FR, t0 + i),
                    v_copy, 0, nf - t0)

        def v_solo(i, carry):
            v_copy(i).start(priority=1)
            return carry

        lax.fori_loop(nf - t0, v_starts[-1], v_solo, 0)

        wait_region(wo_v, sem_w.at[SEM_WO])
        attn = None
        for g in range(H // GH):
            o = jnp.concatenate([o_scr[head_rows(g * GH + j), :] for j in range(GH)], axis=1)
            t = jnp.dot(o.astype(BF16), wo_v[g * GH * Dh:(g + 1) * GH * Dh, :],
                        preferred_element_type=F32)
            attn = t if attn is None else attn + t

        ga, sb, cb, gb = (mod_scr[:, i * D:(i + 1) * D] for i in range(4))
        x1 = x + ga * attn
        h2 = (_layernorm(x1) * (1.0 + cb) + sb).astype(BF16)
        small[2].wait()
        small[3].wait()
        b1 = b1_v[...].astype(F32).reshape(1, F)
        b2 = b2_v[...].astype(F32).reshape(1, D)
        f1 = []
        for sem, lo, hi in ((SEM_W1A, 0, FA), (SEM_W1B, FA, F)):
            wait_region(w1_v.at[pl.ds(lo, hi - lo), :], sem_w.at[sem])
            t = lax.dot_general(h2, w1_v[lo:hi, :], _NT, preferred_element_type=F32) + b1[:, lo:hi]
            f1.append(jax.nn.gelu(t, approximate=True).astype(BF16))
            if lo == 0:
                ft = f1[0][:, VLO:].astype(F32).T
                for b in range(B):
                    fb_scr[b] = jnp.broadcast_to(ft[:, b:b + 1], (FA - VLO, 128))

        parts = [(SEM_W2A, FA, F, f1[1])]
        for p in range(len(W2B)):
            lo, hi = bounds[p], bounds[p + 1]
            parts.append((SEM_W2B + p, lo, hi, f1[0][:, lo:hi]))
        y = b2
        for sem, lo, hi, f in parts:
            wait_region(w2_v.at[pl.ds(lo, hi - lo), :], sem_w.at[sem])
            y = y + jnp.dot(f, w2_v[lo:hi, :], preferred_element_type=F32)
        base = x1 + gb * y

        accs = [None] * B
        for g in range(len(VG)):
            lo, hi = v_starts[g] * VR, v_starts[g + 1] * VR
            wait_region(w2_v.at[pl.ds(VLO + lo, hi - lo), :], sem_w.at[SEM_V + g])
            for r in range(lo, hi, 16):
                w = w2_v[VLO + r:VLO + r + 16, :].astype(F32)
                for b in range(B):
                    p = w * jnp.concatenate([fb_scr[b, r:r + 16, :]] * (D // 128), axis=1)
                    p = p[0:8] + p[8:16]
                    accs[b] = p if accs[b] is None else accs[b] + p
        t = jnp.concatenate([jnp.sum(a, axis=0, keepdims=True) for a in accs], axis=0)
        out_ref[...] = (base + gb * t).astype(out_ref.dtype)

    scratch = [
        pltpu.VMEM((B, D), BF16), pltpu.VMEM((B, D), BF16),
        pltpu.VMEM((F,), BF16), pltpu.VMEM((D,), BF16),
        pltpu.VMEM((D, 6 * D), BF16), pltpu.VMEM((D, H * Dh), BF16),
        pltpu.VMEM((H * Dh, D), BF16), pltpu.VMEM((F, D), BF16), pltpu.VMEM((F, D), BF16),
        pltpu.VMEM((2, NS, GH, R, Dh), BF16),
        pltpu.VMEM((B * H, Dh), F32), pltpu.VMEM((2, CPP, GH, R), F32),
        pltpu.VMEM((2, GH, Dh), F32), pltpu.VMEM((2, GH, Dh), F32),
        pltpu.VMEM((B * H, Dh), F32), pltpu.VMEM((B, 4 * D), F32),
        pltpu.VMEM((B, FA - VLO, 128), F32),
        pltpu.SemaphoreType.DMA((4,)), pltpu.SemaphoreType.DMA((6 + len(W2B) + len(VG),)),
        pltpu.SemaphoreType.DMA((2, NS)),
    ]
    kv_shape = (B, NHALF, GH, 2, Sk, Dh)
    return kernel, scratch, kv_shape


@jax.jit
def pallas_adaLN_cond__sliding_block_cached__dense_activation_gelu__decode_kernel(
    A_x: jax.Array,
    A_k_cache: jax.Array,
    A_v_cache: jax.Array,
    A_wq: jax.Array,
    A_wo: jax.Array,
    B_x: jax.Array,
    B_w1: jax.Array,
    B_b1: jax.Array,
    B_w2: jax.Array,
    B_b2: jax.Array,
    c: jax.Array,
    w_mod: jax.Array,
):
    B, _, D = A_x.shape
    _, H, Sk, Dh = A_k_cache.shape
    F = B_w1.shape[1]
    kernel, scratch, kv_shape = _build(B, D, H, Sk, Dh, F, R=256, LA=6, NS=8, SH=26)
    out = pl.pallas_call(
        kernel,
        in_specs=[pl.BlockSpec(memory_space=pl.ANY)] * 11,
        out_specs=pl.BlockSpec(memory_space=pltpu.VMEM),
        out_shape=jax.ShapeDtypeStruct((B, D), A_x.dtype),
        scratch_shapes=scratch,
        compiler_params=pltpu.CompilerParams(
            vmem_limit_bytes=64 * 1024 * 1024, disable_bounds_checks=True,
            disable_semaphore_checks=True),
    )(A_x.reshape(B, D), A_k_cache.reshape(kv_shape), A_v_cache.reshape(kv_shape),
      A_wq, A_wo, B_w1.T, B_b1, B_w2, B_b2, c, w_mod)
    return out.reshape(B, 1, D)
```

```python
import functools

import jax
import jax.numpy as jnp
from jax import lax
import jax.experimental.pallas as pl
import jax.experimental.pallas.tpu as pltpu

F32 = jnp.float32
BF16 = jnp.bfloat16

_NT = (((1,), (1,)), ((), ()))


def _layernorm(x, eps=1e-5):
    m = jnp.mean(x, axis=-1, keepdims=True)
    d = x - m
    v = jnp.mean(d * d, axis=-1, keepdims=True)
    return d * lax.rsqrt(v + eps)


def _build(B, D, H, Sk, Dh, F, *, R, LA, NS, SH, HN=4, WON=8, WOR=16, FR=32, FN=3,
           W1B=((1504, 4), (1728, 1)), W2B=((384, 4),),
           VG=(6, 5, 4, 3, 3, 3, 2, 2, 1, 1), VR=16):
    W = min(4096, max(256, Sk // 4))
    OFF = Sk - W
    GH = 8
    NHALF = H // (2 * GH)
    NSG = NHALF * B
    CPP = W // R
    NU = NSG * 2 * CPP
    DR = 16
    DPC = R // DR
    ND = NU * DPC
    TR = 8
    FA = F // 2
    n_wo = H * Dh // (2 * WOR)
    scale = float(Dh) ** -0.5
    SHU = -(-SH // DPC)
    assert LA >= SHU and NS > LA and SHU <= CPP and ((LA - SHU + 1) * n_wo) // LA >= SH
    VLO = W2B[-1][0]
    assert FA % (FR * FN) == 0 and VLO + sum(VG) * VR == FA and VLO % 128 == 0

    SEM_WM, SEM_WQ, SEM_WO0, SEM_WO1, SEM_W1A, SEM_W2A, SEM_W1B = range(7)
    SEM_W2B = SEM_W1B + len(W1B)

    def kernel(x_hbm, k_hbm, v_hbm, wq_hbm, wo_hbm, w1_hbm, b1_hbm, w2_hbm, b2_hbm, c_hbm, wm_hbm,
               out_ref,
               x_v, c_v, b1_v, b2_v, wm_v, wq_v, wo_v, w1_v, w2_v, kv_v,
               q_scr, s_scr, l_scr, acc_scr, o_scr, mod_scr, fb_scr,
               sem_s, sem_w, sem_kv):
        small = [pltpu.make_async_copy(x_hbm, x_v, sem_s.at[0]),
                 pltpu.make_async_copy(c_hbm, c_v, sem_s.at[1]),
                 pltpu.make_async_copy(b1_hbm, b1_v, sem_s.at[2]),
                 pltpu.make_async_copy(b2_hbm, b2_v, sem_s.at[3])]

        def wait_region(ref, sem):
            pltpu.make_async_copy(ref, ref, sem).wait()

        def is_v(u):
            return (u // CPP) % 2

        def kv_copy(hbm, th, u, d):
            sg = u // (2 * CPP)
            r0 = pl.multiple_of(OFF + (u % CPP) * R + d * DR, DR)
            d0 = d * DR if isinstance(d, int) else pl.multiple_of(d * DR, DR)
            return pltpu.make_async_copy(
                hbm.at[sg % B, sg // B, :, th, pl.ds(r0, DR), :],
                kv_v.at[th, u % NS, :, pl.ds(d0, DR), :],
                sem_kv.at[th, u % NS])

        def rows_copy(hbm, buf, sem, lo, hi, n, rows, i):
            assert (hi - lo) % (n * rows) == 0
            r0 = pl.multiple_of(lo + (i % n) * ((hi - lo) // n) + (i // n) * rows, TR)
            return pltpu.make_async_copy(hbm.at[pl.ds(r0, rows), :], buf.at[pl.ds(r0, rows), :], sem)

        def wo_copy(th, i):
            half = H * Dh // 2
            return rows_copy(wo_hbm, wo_v, sem_w.at[SEM_WO0 + th], th * half, (th + 1) * half,
                             WON // 2, WOR, i)

        def issue_pairs(f0, f1, lo, hi):
            def step(p, carry):
                f0(p).start(priority=0)
                f1(p).start(priority=1)
                return carry
            lax.fori_loop(lo, hi, step, 0)

        def issue_unit(u):
            runs = {}
            for d in range(DPC):
                du, d0 = divmod(d - SH, DPC)
                runs.setdefault(du, []).append((d, d0))
            for du, pairs in runs.items():
                for v1, hbm1 in enumerate((k_hbm, v_hbm)):
                    for v0, hbm0 in enumerate((k_hbm, v_hbm)):
                        @pl.when(jnp.logical_and(is_v(u) == v1, is_v(u + du) == v0))
                        def _(du=du, pairs=pairs, hbm0=hbm0, hbm1=hbm1):
                            for d, d0 in pairs:
                                kv_copy(hbm0, 0, u + du, d0).start(priority=0)
                                kv_copy(hbm1, 1, u, d).start(priority=1)

        for cp in small:
            cp.start()

        def head_step(t, carry):
            for j in range(2):
                for k in range(HN):
                    r0 = pl.multiple_of(k * (D // HN) + t * TR, TR)
                    for th, (hbm, buf, sem) in enumerate(((wm_hbm, wm_v, sem_w.at[SEM_WM]),
                                                          (wq_hbm, wq_v, sem_w.at[SEM_WQ]))):
                        cw = buf.shape[1] // 2
                        sl = (pl.ds(r0, TR), pl.ds(j * cw, cw))
                        pltpu.make_async_copy(hbm.at[sl], buf.at[sl], sem).start(priority=th)
            return carry

        lax.fori_loop(0, D // (HN * TR), head_step, 0)
        k1_copy = lambda p: kv_copy(k_hbm, 1, p // DPC, p % DPC)
        issue_pairs(functools.partial(wo_copy, 0), k1_copy, 0, SH)
        issue_pairs(lambda p: kv_copy(k_hbm, 0, (p - SH) // DPC, (p - SH) % DPC), k1_copy,
                    SH, SHU * DPC)

        small[0].wait()
        small[1].wait()
        x = x_v[...].astype(F32)
        sc = jax.nn.silu(c_v[...].astype(F32)).astype(BF16)
        wait_region(wm_v, sem_w.at[SEM_WM])
        mod_a = jnp.dot(sc, wm_v[:, 0:2 * D], preferred_element_type=F32)
        h = (_layernorm(x) * (1.0 + mod_a[:, D:2 * D]) + mod_a[:, 0:D]).astype(BF16)

        def prefill(u, carry):
            issue_unit(u)
            return carry

        lax.fori_loop(SHU, LA, prefill, 0)

        def head_rows(hd):
            half, r = divmod(hd, 2 * GH)
            j, th = divmod(r, 2)
            return pl.ds(half * B * 2 * GH + th * GH + j, B, stride=2 * GH)

        def q_proj(g):
            qq = jnp.dot(h, wq_v[:, g * GH * Dh:(g + 1) * GH * Dh], preferred_element_type=F32)
            qq = qq.astype(BF16).astype(F32)
            for j in range(GH):
                q_scr[head_rows(g * GH + j), :] = qq[:, j * Dh:(j + 1) * Dh]

        def mod_rest(i):
            mod_scr[:, 2 * i * D:2 * (i + 1) * D] = jnp.dot(
                sc, wm_v[:, 2 * (i + 1) * D:2 * (i + 2) * D], preferred_element_type=F32)

        wait_region(wq_v, sem_w.at[SEM_WQ])
        q_proj(0)
        q_proj(1)
        acc_scr[...] = jnp.zeros(acc_scr.shape, F32)
        extras = [functools.partial(q_proj, g) for g in range(2, H // GH)]
        extras += [functools.partial(mod_rest, i) for i in range(2)]

        row = lax.broadcasted_iota(jnp.int32, (GH, Dh), 0)

        def unit(u, carry):
            n = u + LA

            @pl.when(n < NU)
            def _():
                issue_unit(n)

            @pl.when(n >= NU)
            def _():
                lo = ((n - NU) * n_wo) // LA
                hi = ((n - NU + 1) * n_wo) // LA
                issue_pairs(lambda p: kv_copy(v_hbm, 0, (ND - SH + p) // DPC, (ND - SH + p) % DPC),
                            functools.partial(wo_copy, 1), lo, jnp.minimum(hi, SH))
                issue_pairs(functools.partial(wo_copy, 0), functools.partial(wo_copy, 1),
                            jnp.maximum(lo, SH), hi)

            slot = u % NS
            cj = u % CPP
            sg = u // (2 * CPP)
            for th in range(2):
                wait_region(kv_v.at[th, slot], sem_kv.at[th, slot])

            @pl.when(is_v(u) == 0)
            def _():
                for th in range(2):
                    qg = q_scr[pl.ds(pl.multiple_of((2 * sg + th) * GH, GH), GH), :]
                    s = None
                    for j in range(GH):
                        qm = jnp.where(row == j, qg, 0.0).astype(BF16)
                        t = lax.dot_general(qm, kv_v[th, slot, j], _NT, preferred_element_type=F32)
                        s = t if s is None else s + t
                    s_scr[th, cj] = s

                @pl.when(cj == CPP - 1)
                def _():
                    for th in range(2):
                        s = s_scr[th] * scale
                        m = jnp.max(jnp.max(s, axis=0), axis=-1, keepdims=True)
                        p = jnp.exp(s - m[None])
                        s_scr[th] = p
                        l = jnp.sum(jnp.sum(p, axis=0), axis=-1, keepdims=True)
                        l_scr[th] = jnp.broadcast_to(l, (GH, Dh))

            @pl.when(is_v(u) == 1)
            def _():
                for th in range(2):
                    p = s_scr[th, cj].astype(BF16)
                    acc = acc_scr[th]
                    for j in range(GH):
                        t = jnp.dot(p, kv_v[th, slot, j], preferred_element_type=F32)
                        acc = acc + jnp.where(row == j, t, 0.0)
                    acc_scr[th] = acc

                @pl.when(cj == CPP - 1)
                def _():
                    for th in range(2):
                        o_scr[pl.ds(pl.multiple_of((2 * sg + th) * GH, GH), GH), :] = (
                            acc_scr[th] / l_scr[th])
                        acc_scr[th] = jnp.zeros((GH, Dh), F32)

            for i, extra in enumerate(extras):
                pl.when(u == i)(extra)
            return carry

        lax.fori_loop(0, NU, unit, 0)

        nf = FA // FR
        bounds1 = (FA,) + tuple(hi for hi, _ in W1B)
        for p, (hi, n) in enumerate(W1B):
            lo = bounds1[p]
            t0 = (lo - FA) // FR
            issue_pairs(
                functools.partial(rows_copy, w1_hbm, w1_v, sem_w.at[SEM_W1A], 0, FA, FN, FR),
                lambda t, p=p, lo=lo, hi=hi, n=n, t0=t0: rows_copy(
                    w1_hbm, w1_v, sem_w.at[SEM_W1B + p], lo, hi, n, FR, t - t0),
                t0, (hi - FA) // FR)

        def wo_proj(th):
            half = H * Dh // 2
            wait_region(wo_v.at[pl.ds(th * half, half), :], sem_w.at[SEM_WO0 + th])
            res = None
            for g in range(th * H // (2 * GH), (th + 1) * H // (2 * GH)):
                o = jnp.concatenate([o_scr[head_rows(g * GH + j), :] for j in range(GH)], axis=1)
                t = jnp.dot(o.astype(BF16), wo_v[g * GH * Dh:(g + 1) * GH * Dh, :],
                            preferred_element_type=F32)
                res = t if res is None else res + t
            return res

        attn = wo_proj(0)
        bounds = (0,) + tuple(hi for hi, _ in W2B)
        for p, (hi, n) in enumerate(W2B):
            lo = bounds[p]
            t0 = lo // FR
            issue_pairs(
                functools.partial(rows_copy, w2_hbm, w2_v, sem_w.at[SEM_W2A], FA, F, FN, FR),
                lambda t, p=p, lo=lo, hi=hi, n=n, t0=t0: rows_copy(
                    w2_hbm, w2_v, sem_w.at[SEM_W2B + p], lo, hi, n, FR, t - t0),
                t0, hi // FR)

        SEM_V = SEM_W2B + len(W2B)
        v_starts = [sum(VG[:g]) for g in range(len(VG) + 1)]

        def v_copy(i):
            g = sum((i >= st).astype(jnp.int32) for st in v_starts[1:-1])
            r0 = pl.multiple_of(VLO + i * VR, TR)
            return pltpu.make_async_copy(w2_hbm.at[pl.ds(r0, VR), :], w2_v.at[pl.ds(r0, VR), :],
                                         sem_w.at[SEM_V + g])

        t0 = VLO // FR
        issue_pairs(lambda i: rows_copy(w2_hbm, w2_v, sem_w.at[SEM_W2A], FA, F, FN, FR, t0 + i),
                    v_copy, 0, nf - t0)

        def v_solo(i, carry):
            v_copy(i).start(priority=1)
            return carry

        lax.fori_loop(nf - t0, v_starts[-1], v_solo, 0)

        attn = attn + wo_proj(1)

        ga, sb, cb, gb = (mod_scr[:, i * D:(i + 1) * D] for i in range(4))
        x1 = x + ga * attn
        h2 = (_layernorm(x1) * (1.0 + cb) + sb).astype(BF16)
        small[2].wait()
        small[3].wait()
        b1 = b1_v[...].astype(F32).reshape(1, F)
        b2 = b2_v[...].astype(F32).reshape(1, D)
        f1 = []
        w1_parts = [(SEM_W1A, 0, FA)]
        w1_parts += [(SEM_W1B + p, bounds1[p], bounds1[p + 1]) for p in range(len(W1B))]
        for sem, lo, hi in w1_parts:
            wait_region(w1_v.at[pl.ds(lo, hi - lo), :], sem_w.at[sem])
            t = lax.dot_general(h2, w1_v[lo:hi, :], _NT, preferred_element_type=F32) + b1[:, lo:hi]
            f1.append(jax.nn.gelu(t, approximate=True).astype(BF16))
            if lo == 0:
                ft = f1[0][:, VLO:].astype(F32).T
                for b in range(B):
                    fb_scr[b] = jnp.broadcast_to(ft[:, b:b + 1], (FA - VLO, 128))

        parts = [(SEM_W2A, FA, F, jnp.concatenate(f1[1:], axis=1))]
        for p in range(len(W2B)):
            lo, hi = bounds[p], bounds[p + 1]
            parts.append((SEM_W2B + p, lo, hi, f1[0][:, lo:hi]))
        y = b2
        for sem, lo, hi, f in parts:
            wait_region(w2_v.at[pl.ds(lo, hi - lo), :], sem_w.at[sem])
            y = y + jnp.dot(f, w2_v[lo:hi, :], preferred_element_type=F32)
        base = x1 + gb * y

        accs = [None] * B
        for g in range(len(VG)):
            lo, hi = v_starts[g] * VR, v_starts[g + 1] * VR
            wait_region(w2_v.at[pl.ds(VLO + lo, hi - lo), :], sem_w.at[SEM_V + g])
            for r in range(lo, hi, 16):
                w = w2_v[VLO + r:VLO + r + 16, :].astype(F32)
                for b in range(B):
                    p = w * jnp.concatenate([fb_scr[b, r:r + 16, :]] * (D // 128), axis=1)
                    p = p[0:8] + p[8:16]
                    accs[b] = p if accs[b] is None else accs[b] + p
        t = jnp.concatenate([jnp.sum(a, axis=0, keepdims=True) for a in accs], axis=0)
        out_ref[...] = (base + gb * t).astype(out_ref.dtype)

    scratch = [
        pltpu.VMEM((B, D), BF16), pltpu.VMEM((B, D), BF16),
        pltpu.VMEM((F,), BF16), pltpu.VMEM((D,), BF16),
        pltpu.VMEM((D, 6 * D), BF16), pltpu.VMEM((D, H * Dh), BF16),
        pltpu.VMEM((H * Dh, D), BF16), pltpu.VMEM((F, D), BF16), pltpu.VMEM((F, D), BF16),
        pltpu.VMEM((2, NS, GH, R, Dh), BF16),
        pltpu.VMEM((B * H, Dh), F32), pltpu.VMEM((2, CPP, GH, R), F32),
        pltpu.VMEM((2, GH, Dh), F32), pltpu.VMEM((2, GH, Dh), F32),
        pltpu.VMEM((B * H, Dh), F32), pltpu.VMEM((B, 4 * D), F32),
        pltpu.VMEM((B, FA - VLO, 128), F32),
        pltpu.SemaphoreType.DMA((4,)), pltpu.SemaphoreType.DMA((6 + len(W1B) + len(W2B) + len(VG),)),
        pltpu.SemaphoreType.DMA((2, NS)),
    ]
    kv_shape = (B, NHALF, GH, 2, Sk, Dh)
    return kernel, scratch, kv_shape


@jax.jit
def pallas_adaLN_cond__sliding_block_cached__dense_activation_gelu__decode_kernel(
    A_x: jax.Array,
    A_k_cache: jax.Array,
    A_v_cache: jax.Array,
    A_wq: jax.Array,
    A_wo: jax.Array,
    B_x: jax.Array,
    B_w1: jax.Array,
    B_b1: jax.Array,
    B_w2: jax.Array,
    B_b2: jax.Array,
    c: jax.Array,
    w_mod: jax.Array,
):
    B, _, D = A_x.shape
    _, H, Sk, Dh = A_k_cache.shape
    F = B_w1.shape[1]
    kernel, scratch, kv_shape = _build(B, D, H, Sk, Dh, F, R=256, LA=6, NS=8, SH=26)
    out = pl.pallas_call(
        kernel,
        in_specs=[pl.BlockSpec(memory_space=pl.ANY)] * 11,
        out_specs=pl.BlockSpec(memory_space=pltpu.VMEM),
        out_shape=jax.ShapeDtypeStruct((B, D), A_x.dtype),
        scratch_shapes=scratch,
        compiler_params=pltpu.CompilerParams(
            vmem_limit_bytes=64 * 1024 * 1024, disable_bounds_checks=True,
            disable_semaphore_checks=True),
    )(A_x.reshape(B, D), A_k_cache.reshape(kv_shape), A_v_cache.reshape(kv_shape),
      A_wq, A_wo, B_w1.T, B_b1, B_w2, B_b2, c, w_mod)
    return out.reshape(B, 1, D)
```

```python
import functools

import jax
import jax.numpy as jnp
from jax import lax
import jax.experimental.pallas as pl
import jax.experimental.pallas.tpu as pltpu

F32 = jnp.float32
BF16 = jnp.bfloat16

_NT = (((1,), (1,)), ((), ()))


def _layernorm(x, eps=1e-5):
    m = jnp.mean(x, axis=-1, keepdims=True)
    d = x - m
    v = jnp.mean(d * d, axis=-1, keepdims=True)
    return d * lax.rsqrt(v + eps)


def _build(B, D, H, Sk, Dh, F, *, R, LA, NS, SH, PRIME=24, HN=4, WON=8, WOR=16, FR=32, FN=3,
           W1B=((1504, 4), (1728, 1)), W2B=((384, 4),),
           VG=(6, 5, 4, 3, 3, 3, 2, 2, 1, 1), VR=16):
    W = min(4096, max(256, Sk // 4))
    OFF = Sk - W
    GH = 8
    NHALF = H // (2 * GH)
    NSG = NHALF * B
    CPP = W // R
    NU = NSG * 2 * CPP
    DR = 16
    DPC = R // DR
    ND = NU * DPC
    TR = 8
    FA = F // 2
    n_wo = H * Dh // (2 * WOR)
    scale = float(Dh) ** -0.5
    SHU = -(-SH // DPC)
    XO = PRIME // 2
    assert PRIME % 2 == 0 and PRIME <= SH
    assert LA >= SHU and NS > LA and SHU <= CPP and ((LA - SHU + 1) * n_wo) // LA >= SH
    VLO = W2B[-1][0]
    assert FA % (FR * FN) == 0 and VLO + sum(VG) * VR == FA and VLO % 128 == 0

    SEM_WM, SEM_WQ, SEM_WO0, SEM_WO1, SEM_W1A, SEM_W2A, SEM_W1B = range(7)
    SEM_W2B = SEM_W1B + len(W1B)

    def kernel(x_hbm, k_hbm, v_hbm, wq_hbm, wo_hbm, w1_hbm, b1_hbm, w2_hbm, b2_hbm, c_hbm, wm_hbm,
               out_ref,
               x_v, c_v, b1_v, b2_v, wm_v, wq_v, wo_v, w1_v, w2_v, kv_v,
               q_scr, s_scr, l_scr, acc_scr, o_scr, mod_scr, fb_scr,
               sem_s, sem_w, sem_kv):
        small = [pltpu.make_async_copy(x_hbm, x_v, sem_s.at[0]),
                 pltpu.make_async_copy(c_hbm, c_v, sem_s.at[1]),
                 pltpu.make_async_copy(b1_hbm, b1_v, sem_s.at[2]),
                 pltpu.make_async_copy(b2_hbm, b2_v, sem_s.at[3])]

        def wait_region(ref, sem):
            pltpu.make_async_copy(ref, ref, sem).wait()

        def is_v(u):
            return (u // CPP) % 2

        def kv_copy(hbm, th, u, d):
            sg = u // (2 * CPP)
            r0 = pl.multiple_of(OFF + (u % CPP) * R + d * DR, DR)
            d0 = d * DR if isinstance(d, int) else pl.multiple_of(d * DR, DR)
            return pltpu.make_async_copy(
                hbm.at[sg % B, sg // B, :, th, pl.ds(r0, DR), :],
                kv_v.at[th, u % NS, :, pl.ds(d0, DR), :],
                sem_kv.at[th, u % NS])

        def rows_copy(hbm, buf, sem, lo, hi, n, rows, i):
            assert (hi - lo) % (n * rows) == 0
            r0 = pl.multiple_of(lo + (i % n) * ((hi - lo) // n) + (i // n) * rows, TR)
            return pltpu.make_async_copy(hbm.at[pl.ds(r0, rows), :], buf.at[pl.ds(r0, rows), :], sem)

        def wo_copy(th, i):
            half = H * Dh // 2
            return rows_copy(wo_hbm, wo_v, sem_w.at[SEM_WO0 + th], th * half, (th + 1) * half,
                             WON // 2, WOR, i)

        def issue_pairs(f0, f1, lo, hi):
            def step(p, carry):
                f0(p).start(priority=0)
                f1(p).start(priority=1)
                return carry
            lax.fori_loop(lo, hi, step, 0)

        def issue_unit(u):
            runs = {}
            for d in range(DPC):
                du, d0 = divmod(d - SH, DPC)
                runs.setdefault(du, []).append((d, d0))
            for du, pairs in runs.items():
                for v1, hbm1 in enumerate((k_hbm, v_hbm)):
                    for v0, hbm0 in enumerate((k_hbm, v_hbm)):
                        @pl.when(jnp.logical_and(is_v(u) == v1, is_v(u + du) == v0))
                        def _(du=du, pairs=pairs, hbm0=hbm0, hbm1=hbm1):
                            for d, d0 in pairs:
                                kv_copy(hbm0, 0, u + du, d0).start(priority=0)
                                kv_copy(hbm1, 1, u, d).start(priority=1)

        def half_copy(hbm, buf, sem, i):
            cw = buf.shape[1] // 2
            sl = (pl.ds(pl.multiple_of((i % HN) * (D // HN) + (i // (2 * HN)) * TR, TR), TR),
                  pl.ds(pl.multiple_of(((i // HN) % 2) * cw, 128), cw))
            return pltpu.make_async_copy(hbm.at[sl], buf.at[sl], sem)

        wm_copy = functools.partial(half_copy, wm_hbm, wm_v, sem_w.at[SEM_WM])
        k0_copy = lambda i: kv_copy(k_hbm, 0, i // DPC, i % DPC)
        k1_copy = lambda i: kv_copy(k_hbm, 1, i // DPC, i % DPC)
        nh = 2 * D // TR

        def step_copy(hbm, buf, sem, t, j, k):
            cw = buf.shape[1] // 2
            sl = (pl.ds(pl.multiple_of(k * (D // HN) + t * TR, TR), TR), pl.ds(j * cw, cw))
            return pltpu.make_async_copy(hbm.at[sl], buf.at[sl], sem)

        PS = PRIME // (2 * HN)
        assert PS * 2 * HN == PRIME

        def prime(t, carry):
            for j in range(2):
                for k in range(HN):
                    step_copy(wq_hbm, wq_v, sem_w.at[SEM_WQ], t, j, k).start(priority=1)
            return carry

        def head_step(t, carry):
            for j in range(2):
                for k in range(HN):
                    step_copy(wm_hbm, wm_v, sem_w.at[SEM_WM], t - PS, j, k).start(priority=0)
                    step_copy(wq_hbm, wq_v, sem_w.at[SEM_WQ], t, j, k).start(priority=1)
            return carry

        lax.fori_loop(0, PS, prime, 0)
        for cp in small:
            cp.start(priority=1)
        lax.fori_loop(PS, D // (HN * TR), head_step, 0)
        issue_pairs(lambda p: wm_copy(p - PRIME), lambda p: k1_copy(p - nh), nh, nh + PRIME)
        issue_pairs(lambda p: wo_copy(0, p - PRIME), k1_copy, PRIME, SH)
        issue_pairs(lambda p: k0_copy(p - SH), k1_copy, SH, SHU * DPC)

        small[0].wait()
        small[1].wait()
        x = x_v[...].astype(F32)
        sc = jax.nn.silu(c_v[...].astype(F32)).astype(BF16)
        wait_region(wm_v, sem_w.at[SEM_WM])
        mod_a = jnp.dot(sc, wm_v[:, 0:2 * D], preferred_element_type=F32)
        h = (_layernorm(x) * (1.0 + mod_a[:, D:2 * D]) + mod_a[:, 0:D]).astype(BF16)

        def prefill(u, carry):
            issue_unit(u)
            return carry

        lax.fori_loop(SHU, LA, prefill, 0)

        def head_rows(hd):
            half, r = divmod(hd, 2 * GH)
            j, th = divmod(r, 2)
            return pl.ds(half * B * 2 * GH + th * GH + j, B, stride=2 * GH)

        def q_proj(g):
            qq = jnp.dot(h, wq_v[:, g * GH * Dh:(g + 1) * GH * Dh], preferred_element_type=F32)
            qq = qq.astype(BF16).astype(F32)
            for j in range(GH):
                q_scr[head_rows(g * GH + j), :] = qq[:, j * Dh:(j + 1) * Dh]

        def mod_rest(i):
            mod_scr[:, 2 * i * D:2 * (i + 1) * D] = jnp.dot(
                sc, wm_v[:, 2 * (i + 1) * D:2 * (i + 2) * D], preferred_element_type=F32)

        wait_region(wq_v, sem_w.at[SEM_WQ])
        q_proj(0)
        q_proj(1)
        acc_scr[...] = jnp.zeros(acc_scr.shape, F32)
        extras = [functools.partial(q_proj, g) for g in range(2, H // GH)]
        extras += [functools.partial(mod_rest, i) for i in range(2)]

        row = lax.broadcasted_iota(jnp.int32, (GH, Dh), 0)

        def unit(u, carry):
            n = u + LA

            @pl.when(n < NU)
            def _():
                issue_unit(n)

            @pl.when(n >= NU)
            def _():
                lo = ((n - NU) * (n_wo + XO)) // LA
                hi = ((n - NU + 1) * (n_wo + XO)) // LA
                v0_copy = lambda p: kv_copy(v_hbm, 0, (ND - SH + p) // DPC, (ND - SH + p) % DPC)
                issue_pairs(v0_copy, lambda p: wo_copy(0, n_wo - XO + p), lo, jnp.minimum(hi, XO))
                issue_pairs(v0_copy, lambda p: wo_copy(1, p - XO),
                            jnp.maximum(lo, XO), jnp.minimum(hi, SH))
                issue_pairs(lambda p: wo_copy(0, p - PRIME), lambda p: wo_copy(1, p - XO),
                            jnp.maximum(lo, SH), hi)

            slot = u % NS
            cj = u % CPP
            sg = u // (2 * CPP)
            for th in range(2):
                wait_region(kv_v.at[th, slot], sem_kv.at[th, slot])

            @pl.when(is_v(u) == 0)
            def _():
                for th in range(2):
                    qg = q_scr[pl.ds(pl.multiple_of((2 * sg + th) * GH, GH), GH), :]
                    s = None
                    for j in range(GH):
                        qm = jnp.where(row == j, qg, 0.0).astype(BF16)
                        t = lax.dot_general(qm, kv_v[th, slot, j], _NT, preferred_element_type=F32)
                        s = t if s is None else s + t
                    s_scr[th, cj] = s

                @pl.when(cj == CPP - 1)
                def _():
                    for th in range(2):
                        s = s_scr[th] * scale
                        m = jnp.max(jnp.max(s, axis=0), axis=-1, keepdims=True)
                        p = jnp.exp(s - m[None])
                        s_scr[th] = p
                        l = jnp.sum(jnp.sum(p, axis=0), axis=-1, keepdims=True)
                        l_scr[th] = jnp.broadcast_to(l, (GH, Dh))

            @pl.when(is_v(u) == 1)
            def _():
                for th in range(2):
                    p = s_scr[th, cj].astype(BF16)
                    acc = acc_scr[th]
                    for j in range(GH):
                        t = jnp.dot(p, kv_v[th, slot, j], preferred_element_type=F32)
                        acc = acc + jnp.where(row == j, t, 0.0)
                    acc_scr[th] = acc

                @pl.when(cj == CPP - 1)
                def _():
                    for th in range(2):
                        o_scr[pl.ds(pl.multiple_of((2 * sg + th) * GH, GH), GH), :] = (
                            acc_scr[th] / l_scr[th])
                        acc_scr[th] = jnp.zeros((GH, Dh), F32)

            for i, extra in enumerate(extras):
                pl.when(u == i)(extra)
            return carry

        lax.fori_loop(0, NU, unit, 0)

        nf = FA // FR
        bounds1 = (FA,) + tuple(hi for hi, _ in W1B)
        for p, (hi, n) in enumerate(W1B):
            lo = bounds1[p]
            t0 = (lo - FA) // FR
            issue_pairs(
                functools.partial(rows_copy, w1_hbm, w1_v, sem_w.at[SEM_W1A], 0, FA, FN, FR),
                lambda t, p=p, lo=lo, hi=hi, n=n, t0=t0: rows_copy(
                    w1_hbm, w1_v, sem_w.at[SEM_W1B + p], lo, hi, n, FR, t - t0),
                t0, (hi - FA) // FR)

        def wo_proj(th):
            half = H * Dh // 2
            wait_region(wo_v.at[pl.ds(th * half, half), :], sem_w.at[SEM_WO0 + th])
            res = None
            for g in range(th * H // (2 * GH), (th + 1) * H // (2 * GH)):
                o = jnp.concatenate([o_scr[head_rows(g * GH + j), :] for j in range(GH)], axis=1)
                t = jnp.dot(o.astype(BF16), wo_v[g * GH * Dh:(g + 1) * GH * Dh, :],
                            preferred_element_type=F32)
                res = t if res is None else res + t
            return res

        attn = wo_proj(0)
        bounds = (0,) + tuple(hi for hi, _ in W2B)
        for p, (hi, n) in enumerate(W2B):
            lo = bounds[p]
            t0 = lo // FR
            issue_pairs(
                functools.partial(rows_copy, w2_hbm, w2_v, sem_w.at[SEM_W2A], FA, F, FN, FR),
                lambda t, p=p, lo=lo, hi=hi, n=n, t0=t0: rows_copy(
                    w2_hbm, w2_v, sem_w.at[SEM_W2B + p], lo, hi, n, FR, t - t0),
                t0, hi // FR)

        SEM_V = SEM_W2B + len(W2B)
        v_starts = [sum(VG[:g]) for g in range(len(VG) + 1)]

        def v_copy(i):
            g = sum((i >= st).astype(jnp.int32) for st in v_starts[1:-1])
            r0 = pl.multiple_of(VLO + i * VR, TR)
            return pltpu.make_async_copy(w2_hbm.at[pl.ds(r0, VR), :], w2_v.at[pl.ds(r0, VR), :],
                                         sem_w.at[SEM_V + g])

        t0 = VLO // FR
        issue_pairs(lambda i: rows_copy(w2_hbm, w2_v, sem_w.at[SEM_W2A], FA, F, FN, FR, t0 + i),
                    v_copy, 0, nf - t0)

        def v_solo(i, carry):
            v_copy(i).start(priority=1)
            return carry

        lax.fori_loop(nf - t0, v_starts[-1], v_solo, 0)

        attn = attn + wo_proj(1)

        ga, sb, cb, gb = (mod_scr[:, i * D:(i + 1) * D] for i in range(4))
        x1 = x + ga * attn
        h2 = (_layernorm(x1) * (1.0 + cb) + sb).astype(BF16)
        small[2].wait()
        small[3].wait()
        b1 = b1_v[...].astype(F32).reshape(1, F)
        b2 = b2_v[...].astype(F32).reshape(1, D)
        f1 = []
        w1_parts = [(SEM_W1A, 0, FA)]
        w1_parts += [(SEM_W1B + p, bounds1[p], bounds1[p + 1]) for p in range(len(W1B))]
        for sem, lo, hi in w1_parts:
            wait_region(w1_v.at[pl.ds(lo, hi - lo), :], sem_w.at[sem])
            t = lax.dot_general(h2, w1_v[lo:hi, :], _NT, preferred_element_type=F32) + b1[:, lo:hi]
            f1.append(jax.nn.gelu(t, approximate=True).astype(BF16))
            if lo == 0:
                ft = f1[0][:, VLO:].astype(F32).T
                for b in range(B):
                    fb_scr[b] = jnp.broadcast_to(ft[:, b:b + 1], (FA - VLO, 128))

        parts = [(SEM_W2A, FA, F, jnp.concatenate(f1[1:], axis=1))]
        for p in range(len(W2B)):
            lo, hi = bounds[p], bounds[p + 1]
            parts.append((SEM_W2B + p, lo, hi, f1[0][:, lo:hi]))
        y = b2
        for sem, lo, hi, f in parts:
            wait_region(w2_v.at[pl.ds(lo, hi - lo), :], sem_w.at[sem])
            y = y + jnp.dot(f, w2_v[lo:hi, :], preferred_element_type=F32)
        base = x1 + gb * y

        accs = [None] * B
        for g in range(len(VG)):
            lo, hi = v_starts[g] * VR, v_starts[g + 1] * VR
            wait_region(w2_v.at[pl.ds(VLO + lo, hi - lo), :], sem_w.at[SEM_V + g])
            for r in range(lo, hi, 16):
                w = w2_v[VLO + r:VLO + r + 16, :].astype(F32)
                for b in range(B):
                    p = w * jnp.concatenate([fb_scr[b, r:r + 16, :]] * (D // 128), axis=1)
                    p = p[0:8] + p[8:16]
                    accs[b] = p if accs[b] is None else accs[b] + p
        t = jnp.concatenate([jnp.sum(a, axis=0, keepdims=True) for a in accs], axis=0)
        out_ref[...] = (base + gb * t).astype(out_ref.dtype)

    scratch = [
        pltpu.VMEM((B, D), BF16), pltpu.VMEM((B, D), BF16),
        pltpu.VMEM((F,), BF16), pltpu.VMEM((D,), BF16),
        pltpu.VMEM((D, 6 * D), BF16), pltpu.VMEM((D, H * Dh), BF16),
        pltpu.VMEM((H * Dh, D), BF16), pltpu.VMEM((F, D), BF16), pltpu.VMEM((F, D), BF16),
        pltpu.VMEM((2, NS, GH, R, Dh), BF16),
        pltpu.VMEM((B * H, Dh), F32), pltpu.VMEM((2, CPP, GH, R), F32),
        pltpu.VMEM((2, GH, Dh), F32), pltpu.VMEM((2, GH, Dh), F32),
        pltpu.VMEM((B * H, Dh), F32), pltpu.VMEM((B, 4 * D), F32),
        pltpu.VMEM((B, FA - VLO, 128), F32),
        pltpu.SemaphoreType.DMA((4,)), pltpu.SemaphoreType.DMA((6 + len(W1B) + len(W2B) + len(VG),)),
        pltpu.SemaphoreType.DMA((2, NS)),
    ]
    kv_shape = (B, NHALF, GH, 2, Sk, Dh)
    return kernel, scratch, kv_shape


@jax.jit
def pallas_adaLN_cond__sliding_block_cached__dense_activation_gelu__decode_kernel(
    A_x: jax.Array,
    A_k_cache: jax.Array,
    A_v_cache: jax.Array,
    A_wq: jax.Array,
    A_wo: jax.Array,
    B_x: jax.Array,
    B_w1: jax.Array,
    B_b1: jax.Array,
    B_w2: jax.Array,
    B_b2: jax.Array,
    c: jax.Array,
    w_mod: jax.Array,
):
    B, _, D = A_x.shape
    _, H, Sk, Dh = A_k_cache.shape
    F = B_w1.shape[1]
    kernel, scratch, kv_shape = _build(B, D, H, Sk, Dh, F, R=256, LA=6, NS=8, SH=26)
    out = pl.pallas_call(
        kernel,
        in_specs=[pl.BlockSpec(memory_space=pl.ANY)] * 11,
        out_specs=pl.BlockSpec(memory_space=pltpu.VMEM),
        out_shape=jax.ShapeDtypeStruct((B, D), A_x.dtype),
        scratch_shapes=scratch,
        compiler_params=pltpu.CompilerParams(
            vmem_limit_bytes=64 * 1024 * 1024, disable_bounds_checks=True,
            disable_semaphore_checks=True),
    )(A_x.reshape(B, D), A_k_cache.reshape(kv_shape), A_v_cache.reshape(kv_shape),
      A_wq, A_wo, B_w1.T, B_b1, B_w2, B_b2, c, w_mod)
    return out.reshape(B, 1, D)
```

```python
import functools

import jax
import jax.numpy as jnp
from jax import lax
import jax.experimental.pallas as pl
import jax.experimental.pallas.tpu as pltpu

F32 = jnp.float32
BF16 = jnp.bfloat16

_NT = (((1,), (1,)), ((), ()))


def _layernorm(x, eps=1e-5):
    m = jnp.mean(x, axis=-1, keepdims=True)
    d = x - m
    v = jnp.mean(d * d, axis=-1, keepdims=True)
    return d * lax.rsqrt(v + eps)


def _build(B, D, H, Sk, Dh, F, *, R, LA, NS, SH, PRIME=24, PRE=4, HN=4, WON=8, WOR=16,
           FR=32, FN=3, W1B=((1504, 4), (1728, 1)), W2B=((384, 4),),
           VG=(6, 5, 4, 3, 3, 3, 2, 2, 1, 1), VR=16):
    W = min(4096, max(256, Sk // 4))
    OFF = Sk - W
    GH = 8
    NHALF = H // (2 * GH)
    NSG = NHALF * B
    CPP = W // R
    NU = NSG * 2 * CPP
    DR = 16
    DPC = R // DR
    ND = NU * DPC
    TR = 8
    FA = F // 2
    n_wo = H * Dh // (2 * WOR)
    scale = float(Dh) ** -0.5
    SHU = -(-SH // DPC)
    XO = PRIME // 2
    assert PRIME % 2 == 0 and PRIME <= SH and SHU <= PRE <= LA
    assert LA >= SHU and NS > LA and SHU <= CPP and ((LA - SHU + 1) * n_wo) // LA >= SH
    VLO = W2B[-1][0]
    assert FA % (FR * FN) == 0 and VLO + sum(VG) * VR == FA and VLO % 128 == 0

    SEM_WM, SEM_WQ, SEM_WO0, SEM_WO1, SEM_W1A, SEM_W2A, SEM_W1B = range(7)
    SEM_W2B = SEM_W1B + len(W1B)

    def kernel(x_hbm, k_hbm, v_hbm, wq_hbm, wo_hbm, w1_hbm, b1_hbm, w2_hbm, b2_hbm, c_hbm, wm_hbm,
               out_ref,
               x_v, c_v, b1_v, b2_v, wm_v, wq_v, wo_v, w1_v, w2_v, kv_v,
               q_scr, s_scr, l_scr, acc_scr, o_scr, mod_scr, fb_scr,
               sem_s, sem_w, sem_kv):
        small = [pltpu.make_async_copy(x_hbm, x_v, sem_s.at[0]),
                 pltpu.make_async_copy(c_hbm, c_v, sem_s.at[1]),
                 pltpu.make_async_copy(b1_hbm, b1_v, sem_s.at[2]),
                 pltpu.make_async_copy(b2_hbm, b2_v, sem_s.at[3])]

        def wait_region(ref, sem):
            pltpu.make_async_copy(ref, ref, sem).wait()

        def is_v(u):
            return (u // CPP) % 2

        def kv_copy(hbm, th, u, d):
            sg = u // (2 * CPP)
            r0 = pl.multiple_of(OFF + (u % CPP) * R + d * DR, DR)
            d0 = d * DR if isinstance(d, int) else pl.multiple_of(d * DR, DR)
            return pltpu.make_async_copy(
                hbm.at[sg % B, sg // B, :, th, pl.ds(r0, DR), :],
                kv_v.at[th, u % NS, :, pl.ds(d0, DR), :],
                sem_kv.at[th, u % NS])

        def rows_copy(hbm, buf, sem, lo, hi, n, rows, i):
            assert (hi - lo) % (n * rows) == 0
            r0 = pl.multiple_of(lo + (i % n) * ((hi - lo) // n) + (i // n) * rows, TR)
            return pltpu.make_async_copy(hbm.at[pl.ds(r0, rows), :], buf.at[pl.ds(r0, rows), :], sem)

        def wo_copy(th, i):
            half = H * Dh // 2
            return rows_copy(wo_hbm, wo_v, sem_w.at[SEM_WO0 + th], th * half, (th + 1) * half,
                             WON // 2, WOR, i)

        def issue_pairs(f0, f1, lo, hi):
            def step(p, carry):
                f0(p).start(priority=0)
                f1(p).start(priority=1)
                return carry
            lax.fori_loop(lo, hi, step, 0)

        def issue_unit(u):
            runs = {}
            for d in range(DPC):
                du, d0 = divmod(d - SH, DPC)
                runs.setdefault(du, []).append((d, d0))
            for du, pairs in runs.items():
                for v1, hbm1 in enumerate((k_hbm, v_hbm)):
                    for v0, hbm0 in enumerate((k_hbm, v_hbm)):
                        @pl.when(jnp.logical_and(is_v(u) == v1, is_v(u + du) == v0))
                        def _(du=du, pairs=pairs, hbm0=hbm0, hbm1=hbm1):
                            for d, d0 in pairs:
                                kv_copy(hbm0, 0, u + du, d0).start(priority=0)
                                kv_copy(hbm1, 1, u, d).start(priority=1)

        def half_copy(hbm, buf, sem, i):
            cw = buf.shape[1] // 2
            sl = (pl.ds(pl.multiple_of((i % HN) * (D // HN) + (i // (2 * HN)) * TR, TR), TR),
                  pl.ds(pl.multiple_of(((i // HN) % 2) * cw, 128), cw))
            return pltpu.make_async_copy(hbm.at[sl], buf.at[sl], sem)

        wm_copy = functools.partial(half_copy, wm_hbm, wm_v, sem_w.at[SEM_WM])
        k0_copy = lambda i: kv_copy(k_hbm, 0, i // DPC, i % DPC)
        k1_copy = lambda i: kv_copy(k_hbm, 1, i // DPC, i % DPC)
        nh = 2 * D // TR

        def step_copy(hbm, buf, sem, t, j, k):
            cw = buf.shape[1] // 2
            sl = (pl.ds(pl.multiple_of(k * (D // HN) + t * TR, TR), TR), pl.ds(j * cw, cw))
            return pltpu.make_async_copy(hbm.at[sl], buf.at[sl], sem)

        PS = PRIME // (2 * HN)
        assert PS * 2 * HN == PRIME

        def prime(t, carry):
            for j in range(2):
                for k in range(HN):
                    step_copy(wq_hbm, wq_v, sem_w.at[SEM_WQ], t, j, k).start(priority=1)
            return carry

        def head_step(t, carry):
            for j in range(2):
                for k in range(HN):
                    step_copy(wm_hbm, wm_v, sem_w.at[SEM_WM], t - PS, j, k).start(priority=0)
                    step_copy(wq_hbm, wq_v, sem_w.at[SEM_WQ], t, j, k).start(priority=1)
            return carry

        lax.fori_loop(0, PS, prime, 0)
        for cp in small:
            cp.start(priority=1)
        lax.fori_loop(PS, D // (HN * TR), head_step, 0)
        issue_pairs(lambda p: wm_copy(p - PRIME), lambda p: k1_copy(p - nh), nh, nh + PRIME)
        issue_pairs(lambda p: wo_copy(0, p - PRIME), k1_copy, PRIME, SH)
        issue_pairs(lambda p: k0_copy(p - SH), k1_copy, SH, SHU * DPC)

        def prefill(u, carry):
            issue_unit(u)
            return carry

        lax.fori_loop(SHU, PRE, prefill, 0)

        small[0].wait()
        small[1].wait()
        x = x_v[...].astype(F32)
        sc = jax.nn.silu(c_v[...].astype(F32)).astype(BF16)
        wait_region(wm_v, sem_w.at[SEM_WM])
        mod_a = jnp.dot(sc, wm_v[:, 0:2 * D], preferred_element_type=F32)
        h = (_layernorm(x) * (1.0 + mod_a[:, D:2 * D]) + mod_a[:, 0:D]).astype(BF16)

        lax.fori_loop(PRE, LA, prefill, 0)

        def head_rows(hd):
            half, r = divmod(hd, 2 * GH)
            j, th = divmod(r, 2)
            return pl.ds(half * B * 2 * GH + th * GH + j, B, stride=2 * GH)

        def q_proj(g):
            qq = jnp.dot(h, wq_v[:, g * GH * Dh:(g + 1) * GH * Dh], preferred_element_type=F32)
            qq = qq.astype(BF16).astype(F32)
            for j in range(GH):
                q_scr[head_rows(g * GH + j), :] = qq[:, j * Dh:(j + 1) * Dh]

        def mod_rest(i):
            mod_scr[:, 2 * i * D:2 * (i + 1) * D] = jnp.dot(
                sc, wm_v[:, 2 * (i + 1) * D:2 * (i + 2) * D], preferred_element_type=F32)

        wait_region(wq_v, sem_w.at[SEM_WQ])
        q_proj(0)
        q_proj(1)
        acc_scr[...] = jnp.zeros(acc_scr.shape, F32)
        extras = [functools.partial(q_proj, g) for g in range(2, H // GH)]
        extras += [functools.partial(mod_rest, i) for i in range(2)]

        row = lax.broadcasted_iota(jnp.int32, (GH, Dh), 0)

        def unit(u, carry):
            n = u + LA

            @pl.when(n < NU)
            def _():
                issue_unit(n)

            @pl.when(n >= NU)
            def _():
                lo = ((n - NU) * (n_wo + XO)) // LA
                hi = ((n - NU + 1) * (n_wo + XO)) // LA
                v0_copy = lambda p: kv_copy(v_hbm, 0, (ND - SH + p) // DPC, (ND - SH + p) % DPC)
                issue_pairs(v0_copy, lambda p: wo_copy(0, n_wo - XO + p), lo, jnp.minimum(hi, XO))
                issue_pairs(v0_copy, lambda p: wo_copy(1, p - XO),
                            jnp.maximum(lo, XO), jnp.minimum(hi, SH))
                issue_pairs(lambda p: wo_copy(0, p - PRIME), lambda p: wo_copy(1, p - XO),
                            jnp.maximum(lo, SH), hi)

            slot = u % NS
            cj = u % CPP
            sg = u // (2 * CPP)
            for th in range(2):
                wait_region(kv_v.at[th, slot], sem_kv.at[th, slot])

            @pl.when(is_v(u) == 0)
            def _():
                for th in range(2):
                    qg = q_scr[pl.ds(pl.multiple_of((2 * sg + th) * GH, GH), GH), :]
                    s = None
                    for j in range(GH):
                        qm = jnp.where(row == j, qg, 0.0).astype(BF16)
                        t = lax.dot_general(qm, kv_v[th, slot, j], _NT, preferred_element_type=F32)
                        s = t if s is None else s + t
                    s_scr[th, cj] = s

                @pl.when(cj == CPP - 1)
                def _():
                    for th in range(2):
                        s = s_scr[th] * scale
                        m = jnp.max(jnp.max(s, axis=0), axis=-1, keepdims=True)
                        p = jnp.exp(s - m[None])
                        s_scr[th] = p
                        l = jnp.sum(jnp.sum(p, axis=0), axis=-1, keepdims=True)
                        l_scr[th] = jnp.broadcast_to(l, (GH, Dh))

            @pl.when(is_v(u) == 1)
            def _():
                for th in range(2):
                    p = s_scr[th, cj].astype(BF16)
                    acc = acc_scr[th]
                    for j in range(GH):
                        t = jnp.dot(p, kv_v[th, slot, j], preferred_element_type=F32)
                        acc = acc + jnp.where(row == j, t, 0.0)
                    acc_scr[th] = acc

                @pl.when(cj == CPP - 1)
                def _():
                    for th in range(2):
                        o_scr[pl.ds(pl.multiple_of((2 * sg + th) * GH, GH), GH), :] = (
                            acc_scr[th] / l_scr[th])
                        acc_scr[th] = jnp.zeros((GH, Dh), F32)

            for i, extra in enumerate(extras):
                pl.when(u == i)(extra)
            return carry

        lax.fori_loop(0, NU, unit, 0)

        nf = FA // FR
        bounds1 = (FA,) + tuple(hi for hi, _ in W1B)
        for p, (hi, n) in enumerate(W1B):
            lo = bounds1[p]
            t0 = (lo - FA) // FR
            issue_pairs(
                functools.partial(rows_copy, w1_hbm, w1_v, sem_w.at[SEM_W1A], 0, FA, FN, FR),
                lambda t, p=p, lo=lo, hi=hi, n=n, t0=t0: rows_copy(
                    w1_hbm, w1_v, sem_w.at[SEM_W1B + p], lo, hi, n, FR, t - t0),
                t0, (hi - FA) // FR)

        def wo_proj(th):
            half = H * Dh // 2
            wait_region(wo_v.at[pl.ds(th * half, half), :], sem_w.at[SEM_WO0 + th])
            res = None
            for g in range(th * H // (2 * GH), (th + 1) * H // (2 * GH)):
                o = jnp.concatenate([o_scr[head_rows(g * GH + j), :] for j in range(GH)], axis=1)
                t = jnp.dot(o.astype(BF16), wo_v[g * GH * Dh:(g + 1) * GH * Dh, :],
                            preferred_element_type=F32)
                res = t if res is None else res + t
            return res

        attn = wo_proj(0)
        bounds = (0,) + tuple(hi for hi, _ in W2B)
        for p, (hi, n) in enumerate(W2B):
            lo = bounds[p]
            t0 = lo // FR
            issue_pairs(
                functools.partial(rows_copy, w2_hbm, w2_v, sem_w.at[SEM_W2A], FA, F, FN, FR),
                lambda t, p=p, lo=lo, hi=hi, n=n, t0=t0: rows_copy(
                    w2_hbm, w2_v, sem_w.at[SEM_W2B + p], lo, hi, n, FR, t - t0),
                t0, hi // FR)

        SEM_V = SEM_W2B + len(W2B)
        v_starts = [sum(VG[:g]) for g in range(len(VG) + 1)]

        def v_copy(i):
            g = sum((i >= st).astype(jnp.int32) for st in v_starts[1:-1])
            r0 = pl.multiple_of(VLO + i * VR, TR)
            return pltpu.make_async_copy(w2_hbm.at[pl.ds(r0, VR), :], w2_v.at[pl.ds(r0, VR), :],
                                         sem_w.at[SEM_V + g])

        t0 = VLO // FR
        issue_pairs(lambda i: rows_copy(w2_hbm, w2_v, sem_w.at[SEM_W2A], FA, F, FN, FR, t0 + i),
                    v_copy, 0, nf - t0)

        def v_solo(i, carry):
            v_copy(i).start(priority=1)
            return carry

        lax.fori_loop(nf - t0, v_starts[-1], v_solo, 0)

        attn = attn + wo_proj(1)

        ga, sb, cb, gb = (mod_scr[:, i * D:(i + 1) * D] for i in range(4))
        x1 = x + ga * attn
        h2 = (_layernorm(x1) * (1.0 + cb) + sb).astype(BF16)
        small[2].wait()
        small[3].wait()
        b1 = b1_v[...].astype(F32).reshape(1, F)
        b2 = b2_v[...].astype(F32).reshape(1, D)
        f1 = []
        w1_parts = [(SEM_W1A, 0, FA)]
        w1_parts += [(SEM_W1B + p, bounds1[p], bounds1[p + 1]) for p in range(len(W1B))]
        for sem, lo, hi in w1_parts:
            wait_region(w1_v.at[pl.ds(lo, hi - lo), :], sem_w.at[sem])
            t = lax.dot_general(h2, w1_v[lo:hi, :], _NT, preferred_element_type=F32) + b1[:, lo:hi]
            f1.append(jax.nn.gelu(t, approximate=True).astype(BF16))
            if lo == 0:
                ft = f1[0][:, VLO:].astype(F32).T
                for b in range(B):
                    fb_scr[b] = jnp.broadcast_to(ft[:, b:b + 1], (FA - VLO, 128))

        parts = [(SEM_W2A, FA, F, jnp.concatenate(f1[1:], axis=1))]
        for p in range(len(W2B)):
            lo, hi = bounds[p], bounds[p + 1]
            parts.append((SEM_W2B + p, lo, hi, f1[0][:, lo:hi]))
        y = b2
        for sem, lo, hi, f in parts:
            wait_region(w2_v.at[pl.ds(lo, hi - lo), :], sem_w.at[sem])
            y = y + jnp.dot(f, w2_v[lo:hi, :], preferred_element_type=F32)
        base = x1 + gb * y

        accs = [None] * B
        for g in range(len(VG)):
            lo, hi = v_starts[g] * VR, v_starts[g + 1] * VR
            wait_region(w2_v.at[pl.ds(VLO + lo, hi - lo), :], sem_w.at[SEM_V + g])
            for r in range(lo, hi, 16):
                w = w2_v[VLO + r:VLO + r + 16, :].astype(F32)
                for b in range(B):
                    p = w * jnp.concatenate([fb_scr[b, r:r + 16, :]] * (D // 128), axis=1)
                    p = p[0:8] + p[8:16]
                    accs[b] = p if accs[b] is None else accs[b] + p
        t = jnp.concatenate([jnp.sum(a, axis=0, keepdims=True) for a in accs], axis=0)
        out_ref[...] = (base + gb * t).astype(out_ref.dtype)

    scratch = [
        pltpu.VMEM((B, D), BF16), pltpu.VMEM((B, D), BF16),
        pltpu.VMEM((F,), BF16), pltpu.VMEM((D,), BF16),
        pltpu.VMEM((D, 6 * D), BF16), pltpu.VMEM((D, H * Dh), BF16),
        pltpu.VMEM((H * Dh, D), BF16), pltpu.VMEM((F, D), BF16), pltpu.VMEM((F, D), BF16),
        pltpu.VMEM((2, NS, GH, R, Dh), BF16),
        pltpu.VMEM((B * H, Dh), F32), pltpu.VMEM((2, CPP, GH, R), F32),
        pltpu.VMEM((2, GH, Dh), F32), pltpu.VMEM((2, GH, Dh), F32),
        pltpu.VMEM((B * H, Dh), F32), pltpu.VMEM((B, 4 * D), F32),
        pltpu.VMEM((B, FA - VLO, 128), F32),
        pltpu.SemaphoreType.DMA((4,)), pltpu.SemaphoreType.DMA((6 + len(W1B) + len(W2B) + len(VG),)),
        pltpu.SemaphoreType.DMA((2, NS)),
    ]
    kv_shape = (B, NHALF, GH, 2, Sk, Dh)
    return kernel, scratch, kv_shape


@jax.jit
def pallas_adaLN_cond__sliding_block_cached__dense_activation_gelu__decode_kernel(
    A_x: jax.Array,
    A_k_cache: jax.Array,
    A_v_cache: jax.Array,
    A_wq: jax.Array,
    A_wo: jax.Array,
    B_x: jax.Array,
    B_w1: jax.Array,
    B_b1: jax.Array,
    B_w2: jax.Array,
    B_b2: jax.Array,
    c: jax.Array,
    w_mod: jax.Array,
):
    B, _, D = A_x.shape
    _, H, Sk, Dh = A_k_cache.shape
    F = B_w1.shape[1]
    kernel, scratch, kv_shape = _build(B, D, H, Sk, Dh, F, R=256, LA=6, NS=8, SH=26)
    out = pl.pallas_call(
        kernel,
        in_specs=[pl.BlockSpec(memory_space=pl.ANY)] * 11,
        out_specs=pl.BlockSpec(memory_space=pltpu.VMEM),
        out_shape=jax.ShapeDtypeStruct((B, D), A_x.dtype),
        scratch_shapes=scratch,
        compiler_params=pltpu.CompilerParams(
            vmem_limit_bytes=64 * 1024 * 1024, disable_bounds_checks=True,
            disable_semaphore_checks=True),
    )(A_x.reshape(B, D), A_k_cache.reshape(kv_shape), A_v_cache.reshape(kv_shape),
      A_wq, A_wo, B_w1.T, B_b1, B_w2, B_b2, c, w_mod)
    return out.reshape(B, 1, D)
```
